```python
import jax
import jax.numpy as jnp

def _softmax(x, axis=-1):
    return jax.nn.softmax(x, axis=axis)
def _gelu(x):
    return jax.nn.gelu(x, approximate=True)
def _silu(x):
    return jax.nn.silu(x)
def _sigmoid(x):
    return jax.nn.sigmoid(x)
def _layernorm(x, axis=-1, eps=1e-5):
    m = jnp.mean(x, axis=axis, keepdims=True)
    v = jnp.var(x, axis=axis, keepdims=True)
    return (x - m) / jnp.sqrt(v + eps)
def _scatter_add(tgt, idx, src, axis=0):
    return tgt.at[idx].add(src)
def _segment_sum(src, seg, n):
    return jax.ops.segment_sum(src, seg, n)
class _Rng:
    def __init__(self, key):
        self._k = key
    def _next(self):
        self._k, sub = jax.random.split(self._k)
        return sub
    def normal(self, shape):
        return jax.random.normal(self._next(), shape, dtype=jnp.bfloat16)
    def randint(self, lo, hi, shape):
        return jax.random.randint(self._next(), shape, lo, hi, dtype=jnp.int32)
    def uniform(self, shape, lo=0.0, hi=1.0):
        return jax.random.uniform(self._next(), shape, jnp.bfloat16, lo, hi)
    def permutation(self, n):
        return jax.random.permutation(self._next(), n)


kernel_name = 'gated_mix__linear_attn_block__moe_arch_mod__prompt'

def setup_inputs():
    _rng = _Rng(jax.random.key(int.from_bytes(__import__("os").urandom(4), "little")))
    _w = (lambda a: (lambda t: t.astype(jnp.bfloat16) if jnp.issubdtype(t.dtype, jnp.floating) else t)(jnp.asarray(a)))
    def _A_setup():
        B, S, D = 1, 2048, 1024
        return {
            "x": _w((lambda *s: _rng.normal(s) * 0.05)(B, S, D)),
            "wqkv": _w((lambda *s: _rng.normal(s) * 0.05)(D, 3 * D)),
            "wo": _w((lambda *s: _rng.normal(s) * 0.05)(D, D)),
        }
    _A_in = _A_setup()

    def _B_setup():
        B, S, D, F, C = 1, 2048, 1024, 3584, 1
        return {
            "x": _w((lambda *s: _rng.normal(s) * 0.05)(B, S, D)),
            "w_r": _w((lambda *s: _rng.normal(s) * 0.05)(D)),
            "w_gate": _w((lambda *s: _rng.normal(s) * 0.05)(D, F)),
            "w_up": _w((lambda *s: _rng.normal(s) * 0.05)(D, F)),
            "w_down": _w((lambda *s: _rng.normal(s) * 0.05)(F, D)),
        }
    _B_in = _B_setup()

    return {
        "A_x": _A_in["x"],
        "A_wqkv": _A_in["wqkv"],
        "A_wo": _A_in["wo"],
        "B_x": _B_in["x"],
        "B_w_r": _B_in["w_r"],
        "B_w_gate": _B_in["w_gate"],
        "B_w_up": _B_in["w_up"],
        "B_w_down": _B_in["w_down"],
        "gate_w": _w((lambda *s: _rng.normal(s) * 0.05)(1024)),
    }

def reference(A_x, A_wqkv, A_wo, B_x, B_w_r, B_w_gate, B_w_up, B_w_down, gate_w):
    def _A_ref(x, wqkv, wo):
        B, S, D = x.shape
        H = 32; Dh = D // H
        qkv = (lambda x, *d: x.transpose(*d))((x @ wqkv).reshape(B, S, 3, H, Dh), 2, 0, 3, 1, 4)
        q, k, v = qkv[0], qkv[1], qkv[2]
        phi = lambda t: jnp.where(t > 0, t + 1, jnp.exp(t)) + 1e-6
        pq, pk = phi(q), phi(k)
        kv = jnp.einsum("bhsd,bhse->bhde", pk, v)
        z = jnp.einsum("bhsd->bhd", pk)
        num = jnp.einsum("bhqd,bhde->bhqe", pq, kv)
        den = jnp.einsum("bhqd,bhd->bhq", pq, z)[..., None] + 1e-6
        o = num / den
        return (lambda x, *d: x.transpose(*d))(o, 0, 2, 1, 3).reshape(B, S, D) @ wo

    def _B_ref(x, w_r, w_gate, w_up, w_down):
        B, S, D = x.shape
        C = 1
        r = x @ w_r
        idx = jnp.argsort(-r, axis=-1)[:, :C]
        idx_e = jnp.repeat(idx.reshape(B, C, 1), D, axis=2)
        x_sel = jnp.take_along_axis(x, idx_e, axis=1)
        g = _silu(x_sel @ w_gate)
        u = x_sel @ w_up
        y = (g * u) @ w_down
        r_sel = _sigmoid(jnp.take_along_axis(r, idx, axis=1))
        y = y * r_sel.reshape(B, C, 1)
        b_off = (jnp.arange(B) * S).reshape(B, 1)
        flat_idx = (idx + b_off).reshape(B * C)
        zero = (x * 0.0).reshape(B * S, D)
        upd = _scatter_add(zero, flat_idx, y.reshape(B * C, D), axis=0)
        return x + upd.reshape(B, S, D)

    x = A_x
    g = _sigmoid((x * gate_w).sum(-1, keepdims=True))
    a = _A_ref(x, A_wqkv, A_wo)
    b = _B_ref(x, B_w_r, B_w_gate, B_w_up, B_w_down)
    return g * a + (1 - g) * b
```

```python
import functools

import jax
import jax.numpy as jnp
from jax import lax
import jax.experimental.pallas as pl
import jax.experimental.pallas.tpu as pltpu

S, D, F = 2048, 1024, 3584
DH = 32
G = 256
NG = D // G
CS = 512
NC = S // CS
T = 256
NT = S // T
XR = 16
FT = 10
FS = 9
NF = 3
LANES = 128

_NT = (((1,), (1,)), ((), ()))
F32, BF16 = jnp.float32, jnp.bfloat16


def _phi(t):
    return jnp.where(t > 0, t + 1.0, jnp.exp(t)) + 1e-6


def _sigmoid(t):
    return 1.0 / (1.0 + jnp.exp(-t))


def _lane_tile_sum(v):
    acc = v[:, 0:LANES]
    for j in range(1, v.shape[1] // LANES):
        acc = acc + v[:, j * LANES:(j + 1) * LANES]
    return acc


def _to_cols(row):
    return jnp.broadcast_to(row, (LANES, row.shape[1])).T


def _matvec(col_ref, k0, w_ref, kk, ntiles):
    accs = [None] * ntiles
    for kb in range(kk // 16):
        c = col_ref[pl.ds(k0 + kb * 16, 16), :]
        for j in range(ntiles):
            w = w_ref[pl.ds(kb * 16, 16), pl.ds(j * LANES, LANES)].astype(F32)
            p = w * c
            p = p[0:8] + p[8:16]
            accs[j] = p if accs[j] is None else accs[j] + p
    return jnp.concatenate(accs, axis=1)


def _kernel(x_hbm, wqkv_hbm, wo_hbm, wr_ref, gw_ref, wg_hbm, wu_hbm, wd_hbm, out_hbm,
            x_v, wk_v, wq_v, wv_v, wo_v, wg_v, wu_v, wd_v,
            wt_v, pk_v, pq_v, pn_v, m_v, gcol_v, xcol_v, hcol_v, y_v, rg_v, ob_v,
            idx_s, sem_x, sem_w, sem_f, sem_o):

    def x_copy(c):
        return pltpu.make_async_copy(x_hbm.at[pl.ds(c * CS, CS)], x_v.at[pl.ds(c * CS, CS)],
                                     sem_x.at[c])

    def w_copy(kind, g):
        off = pl.multiple_of(g * G, G) if not isinstance(g, int) else g * G
        if kind == 3:
            return pltpu.make_async_copy(wo_hbm.at[pl.ds(off, G)], wo_v.at[g], sem_w.at[3 * NG + g])
        dst = (wq_v, wk_v, wv_v)[kind]
        return pltpu.make_async_copy(wqkv_hbm.at[:, pl.ds(kind * D + off, G)], dst.at[g],
                                     sem_w.at[kind * NG + g])

    def f_copy(kind, c):
        off = c * FS * LANES
        if not isinstance(c, int):
            off = pl.multiple_of(off, LANES)
        if kind == 2:
            return pltpu.make_async_copy(wd_hbm.at[pl.ds(off, FT * LANES)], wd_v.at[c],
                                         sem_f.at[2 * NF + c])
        src, dst = ((wg_hbm, wg_v), (wu_hbm, wu_v))[kind]
        return pltpu.make_async_copy(src.at[:, pl.ds(off, FT * LANES)], dst.at[c],
                                     sem_f.at[kind * NF + c])

    def transpose_w(g):
        wt_v[0:G, :] = wk_v[g].T
        wt_v[G:2 * G, :] = wq_v[g].T

    def project(c, first):
        rows = 2 * G + (XR if first else 0)
        kq = lax.dot_general(wt_v[0:rows, :], x_v[c * CS:(c + 1) * CS, :], _NT,
                             preferred_element_type=F32)
        pk = _phi(kq[0:G])
        pk_v[:, c * CS:(c + 1) * CS] = pk.astype(BF16)
        pq_v[:, c * CS:(c + 1) * CS] = _phi(kq[G:2 * G])
        if first:
            rg_v[:, c * CS:(c + 1) * CS] = kq[2 * G:2 * G + 8]
        return _lane_tile_sum(pk)

    def finish_group(g, zacc):
        z = jnp.sum(zacc, axis=1, keepdims=True)
        p = jnp.dot(pk_v[...], x_v[...], preferred_element_type=F32).astype(BF16)
        for c in range(NC):
            pq = pq_v[:, c * CS:(c + 1) * CS].reshape(G // DH, DH, CS)
            den = jnp.sum(pq * z.reshape(G // DH, DH, 1), axis=1, keepdims=True) + 1e-6
            pn = (pq * (1.0 / den)).reshape(G, CS).astype(BF16)
            pn_v[g, c * CS:(c + 1) * CS, :] = pn.T
        ri = lax.broadcasted_iota(jnp.int32, (LANES, LANES), 0) // DH
        ci = lax.broadcasted_iota(jnp.int32, (LANES, LANES), 1) // DH
        for j in range(G // LANES):
            sl = slice(j * LANES, (j + 1) * LANES)
            kv = jnp.dot(p[sl], wv_v[g, :, sl], preferred_element_type=F32)
            kv = jnp.where(ri == ci, kv, 0.0).astype(BF16)
            m_v[g, sl, :] = jnp.dot(kv, wo_v[g, sl, :], preferred_element_type=F32).astype(BF16)

    def ffn_chunk(c):
        hg = jnp.sum(_matvec(xcol_v, 0, wg_v.at[c], D, FT), axis=0, keepdims=True)
        hu = jnp.sum(_matvec(xcol_v, 0, wu_v.at[c], D, FT), axis=0, keepdims=True)
        h = hg * _sigmoid(hg) * hu
        lane = lax.broadcasted_iota(jnp.int32, h.shape, 1)
        h = jnp.where(jnp.logical_or(c == 0, lane >= (FT - FS) * LANES), h, 0.0)
        hcol_v[...] = _to_cols(h)
        y_v[...] += _matvec(hcol_v, 0, wd_v.at[c], FT * LANES, D // LANES)

    w_copy(1, 0).start()
    w_copy(0, 0).start()
    x_copy(0).start()
    wt_v[2 * G:2 * G + XR, :] = jnp.concatenate(
        [wr_ref[...].astype(F32), gw_ref[...].astype(F32), jnp.zeros((XR - 2, D), F32)],
        axis=0).astype(BF16)
    y_v[...] = jnp.zeros(y_v.shape, F32)
    w_copy(1, 0).wait()
    for c in range(1, NC):
        x_copy(c).start()
    w_copy(0, 0).wait()
    transpose_w(0)
    zacc = None
    for c in range(NC):
        x_copy(c).wait()
        if c == 1:
            w_copy(2, 0).start()
            w_copy(3, 0).start()
            w_copy(1, 1).start()
            w_copy(0, 1).start()
        if c == NC - 1:
            for kind in range(3):
                f_copy(kind, 0).start()
        zc = project(c, True)
        zacc = zc if zacc is None else zacc + zc
    w_copy(2, 0).wait()
    w_copy(3, 0).wait()
    w_copy(2, 1).start()
    w_copy(3, 1).start()
    w_copy(1, 1).wait()
    w_copy(0, 1).wait()

    r = rg_v[0:1, :].astype(BF16).astype(F32)
    pos = lax.broadcasted_iota(jnp.int32, (1, S), 1)
    valid = r == r
    rmax = jnp.max(jnp.where(valid, r, -jnp.inf), axis=1, keepdims=True)
    cand = jnp.logical_and(valid, r == rmax)
    idxv = jnp.min(jnp.where(cand, pos, S).astype(F32), axis=1, keepdims=True).astype(jnp.int32)
    idxv = jnp.where(idxv >= S, 0, idxv)
    r_sel = jnp.sum(jnp.where(pos == idxv, r, 0.0), axis=1, keepdims=True)
    idx = idxv[0, 0]
    idx_s[0] = idx
    base = pl.multiple_of(jnp.clip((idx // 16) * 16, 0, S - 16), 16)
    rows = x_v[pl.ds(base, 16), :].astype(F32)
    rid = lax.broadcasted_iota(jnp.int32, (16, D), 0)
    x_sel = jnp.sum(jnp.where(rid == idx - base, rows, 0.0), axis=0, keepdims=True)
    xcol_v[...] = _to_cols(x_sel)
    gcol_v[...] = _to_cols(_sigmoid(rg_v[1:2, :]))
    w_sel = _sigmoid(r_sel)

    finish_group(0, zacc)
    transpose_w(1)

    def group_body(g, carry):
        @pl.when(g + 1 < NG)
        def _():
            for kind in (1, 0, 2, 3):
                w_copy(kind, g + 1).start()
            for kind in range(3):
                f_copy(kind, g).start()
        for kind in range(3):
            f_copy(kind, g - 1).wait()
        w_copy(2, g).wait()
        w_copy(3, g).wait()
        zacc = None
        for c in range(NC):
            zc = project(c, False)
            zacc = zc if zacc is None else zacc + zc
        ffn_chunk(g - 1)
        finish_group(g, zacc)

        @pl.when(g + 1 < NG)
        def _():
            w_copy(1, g + 1).wait()
            w_copy(0, g + 1).wait()
            transpose_w(g + 1)
        return carry

    lax.fori_loop(1, NG, group_body, 0)

    y_v[0:1, :] = jnp.sum(y_v[...], axis=0, keepdims=True) * w_sel

    def o_copy(t):
        return pltpu.make_async_copy(ob_v.at[t % 2], out_hbm.at[pl.ds(pl.multiple_of(t * T, T), T)],
                                     sem_o.at[t % 2])

    def out_body(t, carry):
        @pl.when(t >= 2)
        def _():
            o_copy(t - 2).wait()
        r0 = pl.multiple_of(t * T, T)
        pn = jnp.concatenate([pn_v[g, pl.ds(r0, T), :] for g in range(NG)], axis=1)
        a = jnp.dot(pn, m_v[...].reshape(D, D), preferred_element_type=F32)
        gate = gcol_v[pl.ds(r0, T), :]
        hit = lax.broadcasted_iota(jnp.int32, (T, LANES), 0) == idx_s[0] - r0
        for j in range(D // LANES):
            sl = slice(j * LANES, (j + 1) * LANES)
            xf = x_v[pl.ds(r0, T), sl].astype(F32)
            b = xf + (xf * 0.0 + jnp.where(hit, y_v[0:1, sl], 0.0))
            ob_v[t % 2, :, sl] = (gate * a[:, sl] + (1.0 - gate) * b).astype(BF16)
        o_copy(t).start()
        return carry

    lax.fori_loop(0, NT, out_body, 0)
    o_copy(NT - 2).wait()
    o_copy(NT - 1).wait()


@jax.jit
def pallas_gated_mix__linear_attn_block__moe_arch_mod__prompt_kernel(
    A_x: jax.Array,
    A_wqkv: jax.Array,
    A_wo: jax.Array,
    B_x: jax.Array,
    B_w_r: jax.Array,
    B_w_gate: jax.Array,
    B_w_up: jax.Array,
    B_w_down: jax.Array,
    gate_w: jax.Array,
):
    del B_x
    hbm = pl.BlockSpec(memory_space=pl.ANY)
    vmem = pl.BlockSpec(memory_space=pltpu.VMEM)
    out = pl.pallas_call(
        _kernel,
        out_shape=jax.ShapeDtypeStruct((S, D), BF16),
        in_specs=[hbm, hbm, hbm, vmem, vmem, hbm, hbm, hbm],
        out_specs=hbm,
        scratch_shapes=[
            pltpu.VMEM((S, D), BF16),
            pltpu.VMEM((NG, D, G), BF16),
            pltpu.VMEM((NG, D, G), BF16),
            pltpu.VMEM((NG, D, G), BF16),
            pltpu.VMEM((NG, G, D), BF16),
            pltpu.VMEM((NF, D, FT * LANES), BF16),
            pltpu.VMEM((NF, D, FT * LANES), BF16),
            pltpu.VMEM((NF, FT * LANES, D), BF16),
            pltpu.VMEM((2 * G + XR, D), BF16),
            pltpu.VMEM((G, S), BF16),
            pltpu.VMEM((G, S), F32),
            pltpu.VMEM((NG, S, G), BF16),
            pltpu.VMEM((NG, G, D), BF16),
            pltpu.VMEM((S, LANES), F32),
            pltpu.VMEM((D, LANES), F32),
            pltpu.VMEM((FT * LANES, LANES), F32),
            pltpu.VMEM((8, D), F32),
            pltpu.VMEM((8, S), F32),
            pltpu.VMEM((2, T, D), BF16),
            pltpu.SMEM((1,), jnp.int32),
            pltpu.SemaphoreType.DMA((NC,)),
            pltpu.SemaphoreType.DMA((4 * NG,)),
            pltpu.SemaphoreType.DMA((3 * NF,)),
            pltpu.SemaphoreType.DMA((2,)),
        ],
        compiler_params=pltpu.CompilerParams(vmem_limit_bytes=110 * 1024 * 1024),
    )(A_x.reshape(S, D), A_wqkv, A_wo, B_w_r.reshape(1, D), gate_w.reshape(1, D),
      B_w_gate, B_w_up, B_w_down)
    return out.reshape(A_x.shape)
```

```python
import functools

import jax
import jax.numpy as jnp
from jax import lax
import jax.experimental.pallas as pl
import jax.experimental.pallas.tpu as pltpu

S, D, F = 2048, 1024, 3584
DH = 32
G = 256
NG = D // G
CS = 512
NC = S // CS
PN = 256
T = 256
NT = S // T
XR = 16
LANES = 128
FT, FS = 10, 9
NF = NG - 1
FD = F // (NT - 1)
X0 = (0, 256, 512, 1024, 2048)

import os
PU = int(os.environ.get('PU', 2)); PK = int(os.environ.get('PK', 1)); PJ = int(os.environ.get('PJ', 4))
SK = int(os.environ.get('SK', 10)); SP = int(os.environ.get('SP', 20)); SO = int(os.environ.get('SO', 8)); ACT = int(os.environ.get('ACT', 3))
SU = int(os.environ.get('SU', 2)); SD = int(os.environ.get('SD', 0))
_NT = (((1,), (1,)), ((), ()))
F32, BF16 = jnp.float32, jnp.bfloat16


def _phi(t):
    return jnp.where(t > 0, t + 1.0, jnp.exp(t)) + 1e-6


def _sigmoid(t):
    return 1.0 / (1.0 + jnp.exp(-t))


def _lane_tile_sum(v):
    acc = v[:, 0:LANES]
    for j in range(1, v.shape[1] // LANES):
        acc = acc + v[:, j * LANES:(j + 1) * LANES]
    return acc


def _to_cols(row):
    return jnp.broadcast_to(row, (LANES, row.shape[1])).T


def _advance(steps, n):
    for _ in range(n):
        next(steps, None)


def _bits(v):
    return pltpu.bitcast(v, jnp.int32)


def _kernel(x_hbm, wqkv_hbm, wo_hbm, wr_ref, gw_ref, wg_hbm, wu_hbm, wd_hbm, out_hbm,
            x_v, wq_v, wk_v, wv_v, wo_v, wg_v, wu_v, wd_v,
            wt_v, pk_v, pq_v, p_v, pn_v, m_v, gcol_v, xcol_v, h_v, hcol_v, y_v, rg_v, ob_v, zero_v,
            idx_s, sem_x, sem_w, sem_f, sem_o):

    def x_copy(c):
        rs = pl.ds(X0[c], X0[c + 1] - X0[c])
        return pltpu.make_async_copy(x_hbm.at[rs], x_v.at[rs], sem_x.at[c])

    def w_copy(kind, g):
        off = g * G if isinstance(g, int) else pl.multiple_of(g * G, G)
        if kind == 3:
            return pltpu.make_async_copy(wo_hbm.at[pl.ds(off, G)], wo_v.at[g], sem_w.at[3 * NG + g])
        return pltpu.make_async_copy(wqkv_hbm.at[:, pl.ds(kind * D + off, G)],
                                     (wq_v, wk_v, wv_v)[kind].at[g], sem_w.at[kind * NG + g])

    def f_copy(kind, c):
        off = c * FS * LANES
        sl = pl.ds(off if isinstance(c, int) else pl.multiple_of(off, LANES), FT * LANES)
        return pltpu.make_async_copy((wg_hbm, wu_hbm)[kind].at[:, sl], (wg_v, wu_v)[kind].at[c],
                                     sem_f.at[kind * NF + c])

    def d_copy(i):
        return pltpu.make_async_copy(wd_hbm.at[pl.ds(i * FD, FD)], wd_v.at[i],
                                     sem_f.at[2 * NF + i])

    def o_copy(i, t):
        return pltpu.make_async_copy(ob_v.at[i % 2], out_hbm.at[pl.ds(pl.multiple_of(t * T, T), T)],
                                     sem_o.at[i % 2])

    def after(lhs, token):
        if token is None:
            return lhs
        t = token & zero_v[...]
        top = _bits(lhs[0:16]) | jnp.concatenate([t] * (lhs.shape[1] // LANES), axis=1)
        return jnp.concatenate([pltpu.bitcast(top, BF16), lhs[16:]], axis=0)

    def project(lhs, rs):
        return lax.dot_general(lhs, x_v[rs, :], _NT, preferred_element_type=F32)

    def p_part(n, token, side=iter(())):
        p = jnp.dot(after(pk_v[...], token), x_v[:, n * PN:(n + 1) * PN], preferred_element_type=F32)
        for j in range(0, PN, LANES):
            _advance(side, SP)
            p_v[:, n * PN + j:n * PN + j + LANES] = p[:, j:j + LANES].astype(BF16)

    def normalize(g, rs, pq, z):
        n = pq.shape[1]
        pq = pq.reshape(G // DH, DH, n)
        den = jnp.sum(pq * z, axis=1, keepdims=True) + 1e-6
        pn = (pq * (1.0 / den)).reshape(G, n).astype(BF16).T
        pn_v[g, rs, :] = pn
        return pn

    def kv_part(g):
        ri = lax.broadcasted_iota(jnp.int32, (LANES, LANES), 0) // DH
        ci = lax.broadcasted_iota(jnp.int32, (LANES, LANES), 1) // DH
        out = []
        for j in range(G // LANES):
            sl = slice(j * LANES, (j + 1) * LANES)
            kv = jnp.dot(p_v[sl, :], wv_v[g, :, sl], preferred_element_type=F32)
            out.append(jnp.where(ri == ci, kv, 0.0).astype(BF16))
        return out

    def m_part(g, kvs):
        for j, kv in enumerate(kvs):
            sl = slice(j * LANES, (j + 1) * LANES)
            m_v[g, sl, :] = jnp.dot(kv, wo_v[g, sl, :], preferred_element_type=F32).astype(BF16)

    def route():
        r = rg_v[0:1, :].astype(BF16).astype(F32)
        pos = lax.broadcasted_iota(jnp.int32, (1, S), 1)
        valid = r == r
        rmax = jnp.max(jnp.where(valid, r, -jnp.inf), axis=1, keepdims=True)
        cand = jnp.logical_and(valid, r == rmax)
        idxv = jnp.min(jnp.where(cand, pos, S).astype(F32), axis=1, keepdims=True).astype(jnp.int32)
        idxv = jnp.where(idxv >= S, 0, idxv)
        r_sel = jnp.sum(jnp.where(pos == idxv, r, 0.0), axis=1, keepdims=True)
        idx = idxv[0, 0]
        idx_s[0] = idx
        base = pl.multiple_of(jnp.clip((idx // 16) * 16, 0, S - 16), 16)
        rows = x_v[pl.ds(base, 16), :].astype(F32)
        rid = lax.broadcasted_iota(jnp.int32, (16, D), 0)
        x_sel = jnp.sum(jnp.where(rid == idx - base, rows, 0.0), axis=0, keepdims=True)
        xcol_v[...] = _to_cols(x_sel)
        return _sigmoid(r_sel)

    def matvec(col_ref, nk, tiles, accs, slow):
        keep = zero_v[...] == 0
        for k in range(0, nk, 16):
            lo, hi = col_ref[k:k + 8, :], col_ref[k + 8:k + 16, :]
            if k % (16 * PK) == 0 and accs[-1] is not None:
                t = accs[-1]
                for _ in range(slow):
                    t = pl.reciprocal(t, approx=True)
                lo, hi = jnp.where(keep, lo, t), jnp.where(keep, hi, t)
            for j, (w_ref, r0, c0) in enumerate(tiles):
                w = w_ref[r0 + k:r0 + k + 16, c0:c0 + LANES].astype(F32)
                p = w[0:8] * lo + w[8:16] * hi
                accs[j] = p if accs[j] is None else accs[j] + p
            yield

    def ffn_up(c):
        for i in range(0, FT, PU):
            accs = [None] * (2 * PU)
            yield from matvec(xcol_v, D, [(w.at[c], 0, (i + u) * LANES)
                                          for u in range(PU) for w in (wg_v, wu_v)], accs, SU)
            for u in range(PU):
                h_v[c * FS + i + u, 0:8, :] = accs[2 * u]
                h_v[c * FS + i + u, 8:16, :] = accs[2 * u + 1]

    def ffn_down(i):
        for u in range(FD // LANES):
            hg = jnp.sum(h_v[i * (FD // LANES) + u, 0:8, :], axis=0, keepdims=True)
            hu = jnp.sum(h_v[i * (FD // LANES) + u, 8:16, :], axis=0, keepdims=True)
            hcol_v[u * LANES:(u + 1) * LANES, :] = _to_cols(hg * _sigmoid(hg) * hu)
        for j0 in range(0, D, LANES * PJ):
            cols = range(j0, j0 + LANES * PJ, LANES)
            accs = [y_v[:, j:j + LANES] for j in cols]
            yield from matvec(hcol_v, FD, [(wd_v.at[i], 0, j) for j in cols], accs, SD)
            for j, acc in zip(cols, accs):
                y_v[:, j:j + LANES] = acc

    nx = len(X0) - 1
    w_copy(1, 0).start()
    x_copy(0).start()
    w_copy(0, 0).start()
    x_copy(1).start()
    wt_v[2 * G:2 * G + XR, :] = jnp.concatenate(
        [wr_ref[...].astype(F32).reshape(1, D), gw_ref[...].astype(F32).reshape(1, D),
         jnp.zeros((XR - 2, D), F32)], axis=0).astype(BF16)
    y_v[...] = jnp.zeros(y_v.shape, F32)
    zero_v[...] = jnp.zeros(zero_v.shape, jnp.int32)
    w_copy(1, 0).wait()
    wt_v[G:2 * G, :] = wk_v[0].T
    later = {0: [x_copy(c) for c in range(2, nx)],
             1: [w_copy(2, 0), w_copy(3, 0), w_copy(1, 1)],
             nx - 1: [w_copy(k, 1) for k in (0, 2, 3)] + [w_copy(1, 2)] + [f_copy(k, 0) for k in range(2)]}
    zacc = None
    for c in range(nx):
        rs = slice(X0[c], X0[c + 1])
        x_copy(c).wait()
        for cp in later.get(c, []):
            cp.start()
        if c == 0:
            k = project(wt_v[G:2 * G + XR, :], rs)
            w_copy(0, 0).wait()
            wt_v[0:G, :] = wq_v[0].T
            q = project(wt_v[0:G, :], rs)
        else:
            qk = project(wt_v[...], rs)
            q, k = qk[0:G], qk[G:]
        pk = _phi(k[0:G])
        pk_v[:, rs] = pk.astype(BF16)
        pq_v[:, rs] = _phi(q)
        rg_v[:, rs] = k[G:G + 8]
        zc = _lane_tile_sum(pk)
        zacc = zc if zacc is None else zacc + zc
    for cp in later[1]:
        cp.wait()
    z = jnp.sum(zacc, axis=1, keepdims=True).reshape(G // DH, DH, 1)
    token = None
    for n in range(D // PN):
        p_part(n, token)
        rs = slice(n * CS, (n + 1) * CS)
        if n == 0:
            w_sel = route()
        gcol_v[rs, :] = _to_cols(_sigmoid(rg_v[1:2, rs]))
        pn = normalize(0, rs, pq_v[:, rs], z)
        token = _bits(pn[CS - 16:, G - LANES:])
    wt_v[G:2 * G, :] = wk_v[1].T
    m_part(0, kv_part(0))

    def group_body(g, carry):
        nxt = jnp.minimum(g + 1, NG - 1)

        @pl.when(g + 1 < NG)
        def _():
            for kind in (0, 2, 3):
                w_copy(kind, g + 1).start()
            for kind in range(2):
                f_copy(kind, g).start()

        @pl.when(g + 2 < NG)
        def _():
            w_copy(1, g + 2).start()

        @pl.when(g == NG - 1)
        def _():
            for i in range(F // FD):
                d_copy(i).start()
        for kind in (0, 2, 3):
            w_copy(kind, g).wait()
        for kind in range(2):
            f_copy(kind, g - 1).wait()

        @pl.when(g + 1 < NG)
        def _():
            w_copy(1, g + 1).wait()

        side = ffn_up(g - 1)
        zacc = None
        for c in range(NC):
            k = project(wt_v[G:2 * G, :], slice(c * CS, (c + 1) * CS))
            for j in range(0, CS, LANES):
                pk = _phi(k[:, j:j + LANES])
                _advance(side, SK)
                pk_v[:, c * CS + j:c * CS + j + LANES] = pk.astype(BF16)
                zacc = pk if zacc is None else zacc + pk
        z = jnp.sum(zacc, axis=1, keepdims=True).reshape(G // DH, DH, 1)
        wt_v[0:G, :] = wq_v[g].T
        for n in range(D // PN):
            p_part(n, None, side)
        _advance(side, FT * D)
        wt_v[G:2 * G, :] = wk_v[nxt].T
        for c in range(NC):
            rs = slice(c * CS, (c + 1) * CS)
            normalize(g, rs, _phi(project(wt_v[0:G, :], rs)), z)
            if c == 1:
                kvs = kv_part(g)
            if c == 2:
                m_part(g, kvs)
        return carry

    lax.fori_loop(1, NG, group_body, 0)

    idx = idx_s[0]
    t_hit = jnp.clip(idx // T, 0, NT - 1)

    def tile_of(i):
        return (t_hit + 1 + i) % NT

    def out_tile(i, y, side=iter(())):
        t = tile_of(i)
        rs = pl.ds(pl.multiple_of(t * T, T), T)
        pn = jnp.concatenate([pn_v[g, rs, :] for g in range(NG)], axis=1)
        gate = gcol_v[rs, :]
        a = jnp.dot(pn, m_v[...].reshape(D, D), preferred_element_type=F32)
        for j in range(D // LANES):
            sl = slice(j * LANES, (j + 1) * LANES)
            xf = x_v[rs, sl].astype(F32)
            upd = xf * 0.0
            if y is not None:
                hit = lax.broadcasted_iota(jnp.int32, (T, LANES), 0) == idx - t * T
                upd = upd + jnp.where(hit, y[:, sl], 0.0)
            _advance(side, SO)
            ob_v[i % 2, :, sl] = (gate * a[:, sl] + (1.0 - gate) * (xf + upd)).astype(BF16)
        _advance(side, F)
        o_copy(i, t).start()

    def out_body(i, carry):
        @pl.when(i >= 2)
        def _():
            o_copy(i - 2, tile_of(i - 2)).wait()
        out_tile(i, None, ffn_down(i))
        return carry

    for i in range(F // FD):
        d_copy(i).wait()
    lax.fori_loop(0, NT - 1, out_body, 0)
    o_copy(NT - 3, tile_of(NT - 3)).wait()
    out_tile(NT - 1, jnp.sum(y_v[...], axis=0, keepdims=True) * w_sel)
    o_copy(NT - 2, tile_of(NT - 2)).wait()
    o_copy(NT - 1, tile_of(NT - 1)).wait()


@jax.jit
def pallas_gated_mix__linear_attn_block__moe_arch_mod__prompt_kernel(
    A_x: jax.Array,
    A_wqkv: jax.Array,
    A_wo: jax.Array,
    B_x: jax.Array,
    B_w_r: jax.Array,
    B_w_gate: jax.Array,
    B_w_up: jax.Array,
    B_w_down: jax.Array,
    gate_w: jax.Array,
):
    del B_x
    hbm = pl.BlockSpec(memory_space=pl.ANY)
    vmem = pl.BlockSpec(memory_space=pltpu.VMEM)
    out = pl.pallas_call(
        _kernel,
        out_shape=jax.ShapeDtypeStruct((S, D), BF16),
        in_specs=[hbm, hbm, hbm, vmem, vmem, hbm, hbm, hbm],
        out_specs=hbm,
        scratch_shapes=[
            pltpu.VMEM((S, D), BF16),
            pltpu.VMEM((NG, D, G), BF16),
            pltpu.VMEM((NG, D, G), BF16),
            pltpu.VMEM((NG, D, G), BF16),
            pltpu.VMEM((NG, G, D), BF16),
            pltpu.VMEM((NF, D, FT * LANES), BF16),
            pltpu.VMEM((NF, D, FT * LANES), BF16),
            pltpu.VMEM((F // FD, FD, D), BF16),
            pltpu.VMEM((2 * G + XR, D), BF16),
            pltpu.VMEM((G, S), BF16),
            pltpu.VMEM((G, S), F32),
            pltpu.VMEM((G, D), BF16),
            pltpu.VMEM((NG, S, G), BF16),
            pltpu.VMEM((NG, G, D), BF16),
            pltpu.VMEM((S, LANES), F32),
            pltpu.VMEM((D, LANES), F32),
            pltpu.VMEM((F // LANES, 16, LANES), F32),
            pltpu.VMEM((FD, LANES), F32),
            pltpu.VMEM((8, D), F32),
            pltpu.VMEM((8, S), F32),
            pltpu.VMEM((2, T, D), BF16),
            pltpu.VMEM((8, LANES), jnp.int32),
            pltpu.SMEM((1,), jnp.int32),
            pltpu.SemaphoreType.DMA((len(X0) - 1,)),
            pltpu.SemaphoreType.DMA((4 * NG,)),
            pltpu.SemaphoreType.DMA((2 * NF + F // FD,)),
            pltpu.SemaphoreType.DMA((2,)),
        ],
        compiler_params=pltpu.CompilerParams(vmem_limit_bytes=110 * 1024 * 1024),
    )(A_x.reshape(S, D), A_wqkv, A_wo, B_w_r, gate_w,
      B_w_gate, B_w_up, B_w_down)
    return out.reshape(A_x.shape)
```

```python
import functools

import jax
import jax.numpy as jnp
from jax import lax
import jax.experimental.pallas as pl
import jax.experimental.pallas.tpu as pltpu

S, D, F = 2048, 1024, 3584
DH = 32
G = 256
NG = D // G
CS = 512
NC = S // CS
PN = 256
import os
T = int(os.environ.get('T', 256))
NT = S // T
XR = 16
LANES = 128
FT, FS = 10, 9
NF = NG - 1
ND = NT - 1
FD = -(-F // (ND * LANES)) * LANES
import os
X0 = tuple(int(v) for v in os.environ.get('X0', '0,256,512,1024,2048').split(','))

import os
PU = int(os.environ.get('PU', 2)); PK = int(os.environ.get('PK', 1)); PJ = int(os.environ.get('PJ', 4))
SK = int(os.environ.get('SK', 10)); SP = int(os.environ.get('SP', 20)); SO = int(os.environ.get('SO', 8)); ACT = int(os.environ.get('ACT', 3))
SU = int(os.environ.get('SU', 2)); SD = int(os.environ.get('SD', 4))
UN = int(os.environ.get('UN', 1)); NB = int(os.environ.get('NB', 2))
SX = int(os.environ.get('SX', 1)); SW = int(os.environ.get('SW', 1)); SL = int(os.environ.get('SL', 1))
_NT = (((1,), (1,)), ((), ()))
F32, BF16 = jnp.float32, jnp.bfloat16


def _phi(t):
    return jnp.where(t > 0, t + 1.0, jnp.exp(t)) + 1e-6


def _sigmoid(t):
    return 1.0 / (1.0 + jnp.exp(-t))


def _lane_tile_sum(v):
    acc = v[:, 0:LANES]
    for j in range(1, v.shape[1] // LANES):
        acc = acc + v[:, j * LANES:(j + 1) * LANES]
    return acc


def _to_cols(row):
    return jnp.broadcast_to(row, (LANES, row.shape[1])).T


def _advance(steps, n):
    for _ in range(n):
        next(steps, None)


class _Split:
    def __init__(self, src, dst, sems, base, parts):
        n = src.shape[0] // parts
        self.copies = [pltpu.make_async_copy(src.at[pl.ds(i * n, n)], dst.at[pl.ds(i * n, n)],
                                             sems.at[base + i]) for i in range(parts)]

    def start(self):
        for cp in self.copies:
            cp.start()

    def wait(self):
        for cp in self.copies:
            cp.wait()


def _bits(v):
    return pltpu.bitcast(v, jnp.int32)


def _kernel(x_hbm, wqkv_hbm, wo_hbm, wr_ref, gw_ref, wg_hbm, wu_hbm, wd_hbm, out_hbm,
            x_v, wq_v, wk_v, wv_v, wo_v, wg_v, wu_v, wd_v,
            wt_v, pk_v, pq_v, p_v, pn_v, m_v, gcol_v, xcol_v, h_v, hcol_v, y_v, rg_v, ob_v, zero_v,
            idx_s, sem_x, sem_0, sem_w, sem_f, sem_o):

    def x_copy(c):
        rs = pl.ds(X0[c], X0[c + 1] - X0[c])
        return _Split(x_hbm.at[rs], x_v.at[rs], sem_x, c * SX, SX)

    def w0_copy(kind):
        return _Split(wqkv_hbm.at[:, pl.ds(kind * D, G)], (wq_v, wk_v)[kind].at[0], sem_0, kind * SW, SW)

    def w_copy(kind, g):
        off = g * G if isinstance(g, int) else pl.multiple_of(g * G, G)
        if kind == 3:
            return pltpu.make_async_copy(wo_hbm.at[pl.ds(off, G)], wo_v.at[g], sem_w.at[3 * NG + g])
        return pltpu.make_async_copy(wqkv_hbm.at[:, pl.ds(kind * D + off, G)],
                                     (wq_v, wk_v, wv_v)[kind].at[g], sem_w.at[kind * NG + g])

    def f_copy(kind, c):
        off = c * FS * LANES
        sl = pl.ds(off if isinstance(c, int) else pl.multiple_of(off, LANES), FT * LANES)
        return pltpu.make_async_copy((wg_hbm, wu_hbm)[kind].at[:, sl], (wg_v, wu_v)[kind].at[c],
                                     sem_f.at[kind * NF + c])

    def d_copy(i):
        n = min(FD, F - i * FD)
        return pltpu.make_async_copy(wd_hbm.at[pl.ds(i * FD, n)], wd_v.at[i, pl.ds(0, n)],
                                     sem_f.at[2 * NF + i])

    def o_copy(i, t):
        return pltpu.make_async_copy(ob_v.at[i % NB], out_hbm.at[pl.ds(pl.multiple_of(t * T, T), T)],
                                     sem_o.at[i % NB])

    def o_last(i, t):
        return _Split(ob_v.at[i % NB], out_hbm.at[pl.ds(pl.multiple_of(t * T, T), T)], sem_o, NB, SL)

    def after(lhs, token):
        if token is None:
            return lhs
        t = token & zero_v[...]
        top = _bits(lhs[0:16]) | jnp.concatenate([t] * (lhs.shape[1] // LANES), axis=1)
        return jnp.concatenate([pltpu.bitcast(top, BF16), lhs[16:]], axis=0)

    def project(lhs, rs):
        return lax.dot_general(lhs, x_v[rs, :], _NT, preferred_element_type=F32)

    def p_part(n, token, side=iter(())):
        p = jnp.dot(after(pk_v[...], token), x_v[:, n * PN:(n + 1) * PN], preferred_element_type=F32)
        for j in range(0, PN, LANES):
            _advance(side, SP)
            p_v[:, n * PN + j:n * PN + j + LANES] = p[:, j:j + LANES].astype(BF16)

    def normalize(g, rs, pq, z):
        n = pq.shape[1]
        pq = pq.reshape(G // DH, DH, n)
        den = jnp.sum(pq * z, axis=1, keepdims=True) + 1e-6
        pn = (pq * (1.0 / den)).reshape(G, n).astype(BF16).T
        pn_v[g, rs, :] = pn
        return pn

    def kv_part(g):
        ri = lax.broadcasted_iota(jnp.int32, (LANES, LANES), 0) // DH
        ci = lax.broadcasted_iota(jnp.int32, (LANES, LANES), 1) // DH
        out = []
        for j in range(G // LANES):
            sl = slice(j * LANES, (j + 1) * LANES)
            kv = jnp.dot(p_v[sl, :], wv_v[g, :, sl], preferred_element_type=F32)
            out.append(jnp.where(ri == ci, kv, 0.0).astype(BF16))
        return out

    def m_part(g, kvs):
        for j, kv in enumerate(kvs):
            sl = slice(j * LANES, (j + 1) * LANES)
            m_v[g, sl, :] = jnp.dot(kv, wo_v[g, sl, :], preferred_element_type=F32).astype(BF16)

    def route():
        r = rg_v[0:1, :].astype(BF16).astype(F32)
        pos = lax.broadcasted_iota(jnp.int32, (1, S), 1)
        valid = r == r
        rmax = jnp.max(jnp.where(valid, r, -jnp.inf), axis=1, keepdims=True)
        cand = jnp.logical_and(valid, r == rmax)
        idxv = jnp.min(jnp.where(cand, pos, S).astype(F32), axis=1, keepdims=True).astype(jnp.int32)
        idxv = jnp.where(idxv >= S, 0, idxv)
        r_sel = jnp.sum(jnp.where(pos == idxv, r, 0.0), axis=1, keepdims=True)
        idx = idxv[0, 0]
        idx_s[0] = idx
        base = pl.multiple_of(jnp.clip((idx // 16) * 16, 0, S - 16), 16)
        rows = x_v[pl.ds(base, 16), :].astype(F32)
        rid = lax.broadcasted_iota(jnp.int32, (16, D), 0)
        x_sel = jnp.sum(jnp.where(rid == idx - base, rows, 0.0), axis=0, keepdims=True)
        xcol_v[...] = _to_cols(x_sel)
        return _sigmoid(r_sel)

    def matvec(col_ref, nk, tiles, accs, slow):
        keep = zero_v[...] == 0
        for k in range(0, nk, 16):
            lo, hi = col_ref[k:k + 8, :], col_ref[k + 8:k + 16, :]
            if k % (16 * PK) == 0 and accs[-1] is not None:
                t = accs[-1]
                for _ in range(slow):
                    t = pl.reciprocal(t, approx=True)
                lo, hi = jnp.where(keep, lo, t), jnp.where(keep, hi, t)
            for j, (w_ref, r0, c0) in enumerate(tiles):
                w = w_ref[r0 + k:r0 + k + 16, c0:c0 + LANES].astype(F32)
                p = w[0:8] * lo + w[8:16] * hi
                accs[j] = p if accs[j] is None else accs[j] + p
            yield

    def ffn_up(c):
        for i in range(0, FT, PU):
            accs = [None] * (2 * PU)
            yield from matvec(xcol_v, D, [(w.at[c], 0, (i + u) * LANES)
                                          for u in range(PU) for w in (wg_v, wu_v)], accs, SU)
            for u in range(PU):
                h_v[c * FS + i + u, 0:8, :] = accs[2 * u]
                h_v[c * FS + i + u, 8:16, :] = accs[2 * u + 1]

    def ffn_down(i):
        for u in range(FD // LANES):
            hg = jnp.sum(h_v[i * (FD // LANES) + u, 0:8, :], axis=0, keepdims=True)
            hu = jnp.sum(h_v[i * (FD // LANES) + u, 8:16, :], axis=0, keepdims=True)
            hcol_v[u * LANES:(u + 1) * LANES, :] = _to_cols(hg * _sigmoid(hg) * hu)
        for j0 in range(0, D, LANES * PJ):
            cols = range(j0, j0 + LANES * PJ, LANES)
            accs = [y_v[:, j:j + LANES] for j in cols]
            yield from matvec(hcol_v, FD, [(wd_v.at[i], 0, j) for j in cols], accs, SD)
            for j, acc in zip(cols, accs):
                y_v[:, j:j + LANES] = acc

    nx = len(X0) - 1
    w0_copy(1).start()
    x_copy(0).start()
    w0_copy(0).start()
    x_copy(1).start()
    wt_v[2 * G:2 * G + XR, :] = jnp.concatenate(
        [wr_ref[...].astype(F32).reshape(1, D), gw_ref[...].astype(F32).reshape(1, D),
         jnp.zeros((XR - 2, D), F32)], axis=0).astype(BF16)
    y_v[...] = jnp.zeros(y_v.shape, F32)
    if ND * FD > F:
        wd_v[ND - 1, F - (ND - 1) * FD:, :] = jnp.zeros((ND * FD - F, D), BF16)
        h_v[F // LANES:] = jnp.zeros(((ND * FD - F) // LANES, 16, LANES), F32)
    zero_v[...] = jnp.zeros(zero_v.shape, jnp.int32)
    w0_copy(1).wait()
    wt_v[G:2 * G, :] = wk_v[0].T
    first = [w_copy(2, 0), w_copy(3, 0), w_copy(1, 1)]
    zacc = None
    for c in range(nx):
        rs = slice(X0[c], X0[c + 1])
        x_copy(c).wait()
        if c == 0:
            for cc in range(2, nx):
                x_copy(cc).start()
        if c == nx - 1:
            for cp in (first + [w_copy(k, 1) for k in (0, 2, 3)] + [w_copy(1, 2)]
                       + [f_copy(k, 0) for k in range(2)]):
                cp.start()
        if c == 0:
            k = project(wt_v[G:2 * G + XR, :], rs)
            w0_copy(0).wait()
            wt_v[0:G, :] = wq_v[0].T
            q = project(wt_v[0:G, :], rs)
        else:
            qk = project(wt_v[...], rs)
            q, k = qk[0:G], qk[G:]
        pk = _phi(k[0:G])
        pk_v[:, rs] = pk.astype(BF16)
        pq_v[:, rs] = _phi(q)
        rg_v[:, rs] = k[G:G + 8]
        zc = _lane_tile_sum(pk)
        zacc = zc if zacc is None else zacc + zc
    for cp in first:
        cp.wait()
    z = jnp.sum(zacc, axis=1, keepdims=True).reshape(G // DH, DH, 1)
    token = None
    for n in range(D // PN):
        p_part(n, token)
        rs = slice(n * CS, (n + 1) * CS)
        if n == 0:
            w_sel = route()
        gcol_v[rs, :] = _to_cols(_sigmoid(rg_v[1:2, rs]))
        pn = normalize(0, rs, pq_v[:, rs], z)
        token = _bits(pn[CS - 16:, G - LANES:])
    wt_v[G:2 * G, :] = wk_v[1].T
    m_part(0, kv_part(0))

    def group_body(g, carry):
        nxt = jnp.minimum(g + 1, NG - 1)

        @pl.when(g + 1 < NG)
        def _():
            for kind in (0, 2, 3):
                w_copy(kind, g + 1).start()
            for kind in range(2):
                f_copy(kind, g).start()

        @pl.when(g + 2 < NG)
        def _():
            w_copy(1, g + 2).start()

        @pl.when(g == NG - 1)
        def _():
            for i in range(ND):
                d_copy(i).start()
        for kind in (0, 2, 3):
            w_copy(kind, g).wait()
        for kind in range(2):
            f_copy(kind, g - 1).wait()

        @pl.when(g + 1 < NG)
        def _():
            w_copy(1, g + 1).wait()

        side = ffn_up(g - 1)
        zacc = None
        for c in range(NC):
            k = project(wt_v[G:2 * G, :], slice(c * CS, (c + 1) * CS))
            for j in range(0, CS, LANES):
                pk = _phi(k[:, j:j + LANES])
                _advance(side, SK)
                pk_v[:, c * CS + j:c * CS + j + LANES] = pk.astype(BF16)
                zacc = pk if zacc is None else zacc + pk
        z = jnp.sum(zacc, axis=1, keepdims=True).reshape(G // DH, DH, 1)
        wt_v[0:G, :] = wq_v[g].T
        for n in range(D // PN):
            p_part(n, None, side)
        _advance(side, FT * D)
        wt_v[G:2 * G, :] = wk_v[nxt].T
        for c in range(NC):
            rs = slice(c * CS, (c + 1) * CS)
            normalize(g, rs, _phi(project(wt_v[0:G, :], rs)), z)
            if c == 1:
                kvs = kv_part(g)
            if c == 2:
                m_part(g, kvs)
        return carry

    lax.fori_loop(1, NG, group_body, 0)

    idx = idx_s[0]
    t_hit = jnp.clip(idx // T, 0, NT - 1)

    def tile_of(i):
        return (t_hit + 1 + i) % NT

    def out_tile(i, y, side=iter(())):
        t = tile_of(i)
        rs = pl.ds(pl.multiple_of(t * T, T), T)
        pn = jnp.concatenate([pn_v[g, rs, :] for g in range(NG)], axis=1)
        gate = gcol_v[rs, :]
        a = jnp.dot(pn, m_v[...].reshape(D, D), preferred_element_type=F32)
        for j in range(D // LANES):
            sl = slice(j * LANES, (j + 1) * LANES)
            xf = x_v[rs, sl].astype(F32)
            upd = xf * 0.0
            if y is not None:
                hit = lax.broadcasted_iota(jnp.int32, (T, LANES), 0) == idx - t * T
                upd = upd + jnp.where(hit, y[:, sl], 0.0)
            _advance(side, SO)
            ob_v[i % NB, :, sl] = (gate * a[:, sl] + (1.0 - gate) * (xf + upd)).astype(BF16)
        _advance(side, F)
        (o_copy if y is None else o_last)(i, t).start()

    def out_step(i):
        if isinstance(i, int):
            if i >= NB:
                o_copy(i - NB, tile_of(i - NB)).wait()
        else:
            @pl.when(i >= NB)
            def _():
                o_copy(i - NB, tile_of(i - NB)).wait()
        out_tile(i, None, ffn_down(i))

    def out_body(ii, carry):
        for u in range(UN):
            out_step(ii * UN + u)
        return carry

    for i in range(ND):
        d_copy(i).wait()
    n_loop = (NT - 1) // UN if UN < NT else 0
    if n_loop:
        lax.fori_loop(0, n_loop, out_body, 0)
    for i in range(n_loop * UN, NT - 1):
        out_step(i)
    o_copy(NT - 1 - NB, tile_of(NT - 1 - NB)).wait()
    out_tile(NT - 1, jnp.sum(y_v[...], axis=0, keepdims=True) * w_sel)
    for i in range(NT - NB, NT - 1):
        o_copy(i, tile_of(i)).wait()
    o_last(NT - 1, tile_of(NT - 1)).wait()


@jax.jit
def pallas_gated_mix__linear_attn_block__moe_arch_mod__prompt_kernel(
    A_x: jax.Array,
    A_wqkv: jax.Array,
    A_wo: jax.Array,
    B_x: jax.Array,
    B_w_r: jax.Array,
    B_w_gate: jax.Array,
    B_w_up: jax.Array,
    B_w_down: jax.Array,
    gate_w: jax.Array,
):
    del B_x
    hbm = pl.BlockSpec(memory_space=pl.ANY)
    vmem = pl.BlockSpec(memory_space=pltpu.VMEM)
    out = pl.pallas_call(
        _kernel,
        out_shape=jax.ShapeDtypeStruct((S, D), BF16),
        in_specs=[hbm, hbm, hbm, vmem, vmem, hbm, hbm, hbm],
        out_specs=hbm,
        scratch_shapes=[
            pltpu.VMEM((S, D), BF16),
            pltpu.VMEM((NG, D, G), BF16),
            pltpu.VMEM((NG, D, G), BF16),
            pltpu.VMEM((NG, D, G), BF16),
            pltpu.VMEM((NG, G, D), BF16),
            pltpu.VMEM((NF, D, FT * LANES), BF16),
            pltpu.VMEM((NF, D, FT * LANES), BF16),
            pltpu.VMEM((ND, FD, D), BF16),
            pltpu.VMEM((2 * G + XR, D), BF16),
            pltpu.VMEM((G, S), BF16),
            pltpu.VMEM((G, S), F32),
            pltpu.VMEM((G, D), BF16),
            pltpu.VMEM((NG, S, G), BF16),
            pltpu.VMEM((NG, G, D), BF16),
            pltpu.VMEM((S, LANES), F32),
            pltpu.VMEM((D, LANES), F32),
            pltpu.VMEM((ND * FD // LANES, 16, LANES), F32),
            pltpu.VMEM((FD, LANES), F32),
            pltpu.VMEM((8, D), F32),
            pltpu.VMEM((8, S), F32),
            pltpu.VMEM((NB, T, D), BF16),
            pltpu.VMEM((8, LANES), jnp.int32),
            pltpu.SMEM((1,), jnp.int32),
            pltpu.SemaphoreType.DMA(((len(X0) - 1) * SX,)),
            pltpu.SemaphoreType.DMA((2 * SW,)),
            pltpu.SemaphoreType.DMA((4 * NG,)),
            pltpu.SemaphoreType.DMA((2 * NF + ND,)),
            pltpu.SemaphoreType.DMA((NB + SL,)),
        ],
        compiler_params=pltpu.CompilerParams(vmem_limit_bytes=110 * 1024 * 1024),
    )(A_x.reshape(S, D), A_wqkv, A_wo, B_w_r, gate_w,
      B_w_gate, B_w_up, B_w_down)
    return out.reshape(A_x.shape)
```

```python
import functools

import jax
import jax.numpy as jnp
from jax import lax
import jax.experimental.pallas as pl
import jax.experimental.pallas.tpu as pltpu

S, D, F = 2048, 1024, 3584
DH = 32
G = 256
NG = D // G
CS = 512
NC = S // CS
PN = 256
import os
T = int(os.environ.get('T', 256))
NT = S // T
XR = 16
LANES = 128
FT, FS = 10, 9
NF = NG - 1
ND = NT - 1
FD = -(-F // (ND * LANES)) * LANES
import os
X0 = tuple(int(v) for v in os.environ.get('X0', '0,256,512,1024,2048').split(','))

import os
PU = int(os.environ.get('PU', 2)); PK = int(os.environ.get('PK', 1)); PJ = int(os.environ.get('PJ', 4))
SK = int(os.environ.get('SK', 10)); SP = int(os.environ.get('SP', 20)); SO = int(os.environ.get('SO', 8)); ACT = int(os.environ.get('ACT', 3))
SU = int(os.environ.get('SU', 2)); SD = int(os.environ.get('SD', 4))
UN = int(os.environ.get('UN', 1)); NB = int(os.environ.get('NB', 2))
SX = int(os.environ.get('SX', 1)); SW = int(os.environ.get('SW', 1)); SL = int(os.environ.get('SL', 1))
DA = int(os.environ.get('DA', 20)); GT = int(os.environ.get('GT', 1)); MR = int(os.environ.get('MR', 0)); MC = int(os.environ.get('MC', 384))
TK = int(os.environ.get('TK', 1))
_NT = (((1,), (1,)), ((), ()))
F32, BF16 = jnp.float32, jnp.bfloat16


def _phi(t):
    return jnp.where(t > 0, t + 1.0, jnp.exp(t)) + 1e-6


def _sigmoid(t):
    return 1.0 / (1.0 + jnp.exp(-t))


def _lane_tile_sum(v):
    acc = v[:, 0:LANES]
    for j in range(1, v.shape[1] // LANES):
        acc = acc + v[:, j * LANES:(j + 1) * LANES]
    return acc


def _to_cols(row):
    return jnp.broadcast_to(row, (LANES, row.shape[1])).T


def _advance(steps, n):
    for _ in range(n):
        next(steps, None)


class _Split:
    def __init__(self, src, dst, sems, base, parts):
        n = src.shape[0] // parts
        self.copies = [pltpu.make_async_copy(src.at[pl.ds(i * n, n)], dst.at[pl.ds(i * n, n)],
                                             sems.at[base + i]) for i in range(parts)]

    def start(self):
        for cp in self.copies:
            cp.start()

    def wait(self):
        for cp in self.copies:
            cp.wait()


def _bits(v):
    return pltpu.bitcast(v, jnp.int32)


def _fold(v, delay=0):
    v = _bits(v)
    v = functools.reduce(jnp.bitwise_or, [v[:, j:j + LANES] for j in range(0, v.shape[1], LANES)])
    v = functools.reduce(jnp.bitwise_or, [v[i:i + 8] for i in range(0, v.shape[0], 8)])
    v = pltpu.bitcast(v, F32)
    for _ in range(delay):
        v = pl.reciprocal(v, approx=True)
    return _bits(v)


def _kernel(x_hbm, wqkv_hbm, wo_hbm, wr_ref, gw_ref, wg_hbm, wu_hbm, wd_hbm, out_hbm,
            x_v, wq_v, wk_v, wv_v, wo_v, wg_v, wu_v, wd_v,
            wt_v, pk_v, pq_v, p_v, pn_v, m_v, gcol_v, xcol_v, h_v, hcol_v, y_v, rg_v, ob_v, zero_v,
            idx_s, sem_x, sem_0, sem_w, sem_f, sem_o):

    def x_copy(c):
        rs = pl.ds(X0[c], X0[c + 1] - X0[c])
        return _Split(x_hbm.at[rs], x_v.at[rs], sem_x, c * SX, SX)

    def w0_copy(kind):
        return _Split(wqkv_hbm.at[:, pl.ds(kind * D, G)], (wq_v, wk_v)[kind].at[0], sem_0, kind * SW, SW)

    def w_copy(kind, g):
        off = g * G if isinstance(g, int) else pl.multiple_of(g * G, G)
        if kind == 3:
            return pltpu.make_async_copy(wo_hbm.at[pl.ds(off, G)], wo_v.at[g], sem_w.at[3 * NG + g])
        return pltpu.make_async_copy(wqkv_hbm.at[:, pl.ds(kind * D + off, G)],
                                     (wq_v, wk_v, wv_v)[kind].at[g], sem_w.at[kind * NG + g])

    def f_copy(kind, c):
        off = c * FS * LANES
        sl = pl.ds(off if isinstance(c, int) else pl.multiple_of(off, LANES), FT * LANES)
        return pltpu.make_async_copy((wg_hbm, wu_hbm)[kind].at[:, sl], (wg_v, wu_v)[kind].at[c],
                                     sem_f.at[kind * NF + c])

    def d_copy(i):
        n = min(FD, F - i * FD)
        return pltpu.make_async_copy(wd_hbm.at[pl.ds(i * FD, n)], wd_v.at[i, pl.ds(0, n)],
                                     sem_f.at[2 * NF + i])

    def o_copy(i, t):
        return pltpu.make_async_copy(ob_v.at[i % NB], out_hbm.at[pl.ds(pl.multiple_of(t * T, T), T)],
                                     sem_o.at[i % NB])

    def o_last(i, t):
        return _Split(ob_v.at[i % NB], out_hbm.at[pl.ds(pl.multiple_of(t * T, T), T)], sem_o, NB, SL)

    def after(lhs, token):
        if token is None:
            return lhs
        t = token & zero_v[...]
        top = _bits(lhs[0:16]) | jnp.concatenate([t] * (lhs.shape[1] // LANES), axis=1)
        return jnp.concatenate([pltpu.bitcast(top, BF16), lhs[16:]], axis=0)

    def project(lhs, rs):
        return lax.dot_general(lhs, x_v[rs, :], _NT, preferred_element_type=F32)

    def p_part(n, token, side=iter(())):
        p = jnp.dot(after(pk_v[...], token), x_v[:, n * PN:(n + 1) * PN], preferred_element_type=F32)
        for j in range(0, PN, LANES):
            _advance(side, SP)
            p_v[:, n * PN + j:n * PN + j + LANES] = p[:, j:j + LANES].astype(BF16)

    def normalize(g, rs, pq, z):
        n = pq.shape[1]
        pq = pq.reshape(G // DH, DH, n)
        den = jnp.sum(pq * z, axis=1, keepdims=True) + 1e-6
        pn = (pq * (1.0 / den)).reshape(G, n).astype(BF16).T
        pn_v[g, rs, :] = pn
        return pn

    def kv_part(g):
        ri = lax.broadcasted_iota(jnp.int32, (LANES, LANES), 0) // DH
        ci = lax.broadcasted_iota(jnp.int32, (LANES, LANES), 1) // DH
        out = []
        for j in range(G // LANES):
            sl = slice(j * LANES, (j + 1) * LANES)
            kv = jnp.dot(p_v[sl, :], wv_v[g, :, sl], preferred_element_type=F32)
            out.append(jnp.where(ri == ci, kv, 0.0).astype(BF16))
        return out

    def m_part(g, kvs, token=None):
        for j, kv in enumerate(kvs):
            sl = slice(j * LANES, (j + 1) * LANES)
            m_v[g, sl, :] = jnp.dot(after(kv, token), wo_v[g, sl, :], preferred_element_type=F32).astype(BF16)

    def route():
        r = rg_v[0:1, :].astype(BF16).astype(F32)
        pos = lax.broadcasted_iota(jnp.int32, (1, S), 1)
        valid = r == r
        rmax = jnp.max(jnp.where(valid, r, -jnp.inf), axis=1, keepdims=True)
        cand = jnp.logical_and(valid, r == rmax)
        idxv = jnp.min(jnp.where(cand, pos, S).astype(F32), axis=1, keepdims=True).astype(jnp.int32)
        idxv = jnp.where(idxv >= S, 0, idxv)
        r_sel = jnp.sum(jnp.where(pos == idxv, r, 0.0), axis=1, keepdims=True)
        idx = idxv[0, 0]
        idx_s[0] = idx
        base = pl.multiple_of(jnp.clip((idx // 16) * 16, 0, S - 16), 16)
        rows = x_v[pl.ds(base, 16), :].astype(F32)
        rid = lax.broadcasted_iota(jnp.int32, (16, D), 0)
        x_sel = jnp.sum(jnp.where(rid == idx - base, rows, 0.0), axis=0, keepdims=True)
        xcol_v[...] = _to_cols(x_sel)
        return _sigmoid(r_sel)

    def matvec(col_ref, nk, tiles, accs, slow):
        keep = zero_v[...] == 0
        for k in range(0, nk, 16):
            lo, hi = col_ref[k:k + 8, :], col_ref[k + 8:k + 16, :]
            if k % (16 * PK) == 0 and accs[-1] is not None:
                t = accs[-1]
                for _ in range(slow):
                    t = pl.reciprocal(t, approx=True)
                lo, hi = jnp.where(keep, lo, t), jnp.where(keep, hi, t)
            for j, (w_ref, r0, c0) in enumerate(tiles):
                w = w_ref[r0 + k:r0 + k + 16, c0:c0 + LANES].astype(F32)
                p = w[0:8] * lo + w[8:16] * hi
                accs[j] = p if accs[j] is None else accs[j] + p
            yield

    def ffn_up(c):
        for i in range(0, FT, PU):
            accs = [None] * (2 * PU)
            yield from matvec(xcol_v, D, [(w.at[c], 0, (i + u) * LANES)
                                          for u in range(PU) for w in (wg_v, wu_v)], accs, SU)
            for u in range(PU):
                h_v[c * FS + i + u, 0:8, :] = accs[2 * u]
                h_v[c * FS + i + u, 8:16, :] = accs[2 * u + 1]

    def ffn_down(i):
        for u in range(FD // LANES):
            hg = jnp.sum(h_v[i * (FD // LANES) + u, 0:8, :], axis=0, keepdims=True)
            hu = jnp.sum(h_v[i * (FD // LANES) + u, 8:16, :], axis=0, keepdims=True)
            hcol_v[u * LANES:(u + 1) * LANES, :] = _to_cols(hg * _sigmoid(hg) * hu)
        for j0 in range(0, D, LANES * PJ):
            cols = range(j0, j0 + LANES * PJ, LANES)
            accs = [y_v[:, j:j + LANES] for j in cols]
            yield from matvec(hcol_v, FD, [(wd_v.at[i], 0, j) for j in cols], accs, SD)
            for j, acc in zip(cols, accs):
                y_v[:, j:j + LANES] = acc

    nx = len(X0) - 1
    w0_copy(1).start()
    x_copy(0).start()
    w0_copy(0).start()
    x_copy(1).start()
    wt_v[2 * G:2 * G + XR, :] = jnp.concatenate(
        [wr_ref[...].astype(F32).reshape(1, D), gw_ref[...].astype(F32).reshape(1, D),
         jnp.zeros((XR - 2, D), F32)], axis=0).astype(BF16)
    y_v[...] = jnp.zeros(y_v.shape, F32)
    if ND * FD > F:
        wd_v[ND - 1, F - (ND - 1) * FD:, :] = jnp.zeros((ND * FD - F, D), BF16)
        h_v[F // LANES:] = jnp.zeros(((ND * FD - F) // LANES, 16, LANES), F32)
    zero_v[...] = jnp.zeros(zero_v.shape, jnp.int32)
    w0_copy(1).wait()
    wt_v[G:2 * G, :] = wk_v[0].T
    first = [w_copy(2, 0), w_copy(3, 0), w_copy(1, 1)]
    zacc = None
    for c in range(nx):
        rs = slice(X0[c], X0[c + 1])
        x_copy(c).wait()
        if c == 0:
            for cc in range(2, nx):
                x_copy(cc).start()
        if c == nx - 1:
            for cp in (first + [w_copy(k, 1) for k in (0, 2, 3)] + [w_copy(1, 2)]
                       + [f_copy(k, 0) for k in range(2)]):
                cp.start()
        if c == 0:
            k = project(wt_v[G:2 * G + XR, :], rs)
            w0_copy(0).wait()
            wt_v[0:G, :] = wq_v[0].T
            q = project(wt_v[0:G, :], rs)
        elif c < nx - 1:
            qk = project(wt_v[...], rs)
            q, k = qk[0:G], qk[G:]
        else:
            q, k = None, project(wt_v[G:2 * G + XR, :], rs)
        pk = _phi(k[0:G])
        pk_v[:, rs] = pk.astype(BF16)
        if q is not None:
            pq_v[:, rs] = _phi(q)
        rg_v[:, rs] = k[G:G + 8]
        zc = _lane_tile_sum(pk)
        zacc = zc if zacc is None else zacc + zc
    for cp in first:
        cp.wait()
    z = jnp.sum(zacc, axis=1, keepdims=True).reshape(G // DH, DH, 1)
    token = None
    for n in range(D // PN):
        p_part(n, token)
        rs = slice(n * CS, (n + 1) * CS)
        if n == 0:
            w_sel = route()
        gcol_v[rs, :] = _to_cols(_sigmoid(rg_v[1:2, rs]))
        token = None
        if (n + 1) * CS <= X0[nx - 1]:
            pn = normalize(0, rs, pq_v[:, rs], z)
            if TK:
                token = _bits(pn[CS - 16:, G - LANES:])
    wt_v[G:2 * G, :] = wk_v[1].T
    kvs = kv_part(0)
    for r0 in range(X0[nx - 1], S, CS):
        rs = slice(r0, r0 + CS)
        q = project(wt_v[0:G, :], rs)
        normalize(0, rs, _phi(q), z)
    m_part(0, kvs, _bits(q[MR:MR + 8, MC:MC + LANES]))

    def group_body(g, carry):
        nxt = jnp.minimum(g + 1, NG - 1)

        @pl.when(g + 1 < NG)
        def _():
            for kind in (0, 2, 3):
                w_copy(kind, g + 1).start()
            for kind in range(2):
                f_copy(kind, g).start()

        @pl.when(g + 2 < NG)
        def _():
            w_copy(1, g + 2).start()

        @pl.when(g == NG - 1)
        def _():
            for i in range(ND):
                d_copy(i).start()
        for kind in (0, 2, 3):
            w_copy(kind, g).wait()
        for kind in range(2):
            f_copy(kind, g - 1).wait()

        @pl.when(g + 1 < NG)
        def _():
            w_copy(1, g + 1).wait()

        side = ffn_up(g - 1)
        zacc = None
        for c in range(NC):
            k = project(wt_v[G:2 * G, :], slice(c * CS, (c + 1) * CS))
            for j in range(0, CS, LANES):
                pk = _phi(k[:, j:j + LANES])
                _advance(side, SK)
                pk_v[:, c * CS + j:c * CS + j + LANES] = pk.astype(BF16)
                zacc = pk if zacc is None else zacc + pk
        z = jnp.sum(zacc, axis=1, keepdims=True).reshape(G // DH, DH, 1)
        wt_v[0:G, :] = wq_v[g].T
        for n in range(D // PN):
            p_part(n, None, side)
        _advance(side, FT * D)
        wt_v[G:2 * G, :] = wk_v[nxt].T
        for c in range(NC):
            rs = slice(c * CS, (c + 1) * CS)
            q = project(wt_v[0:G, :], rs)
            normalize(g, rs, _phi(q), z)
            if c == 1:
                kvs = kv_part(g)
            if c == NC - 1:
                m_part(g, kvs, _bits(q[MR:MR + 8, MC:MC + LANES]) if MC >= 0 else None)
        return carry

    lax.fori_loop(1, NG, group_body, 0)

    idx = idx_s[0]
    t_hit = jnp.clip(idx // T, 0, NT - 1)

    def tile_of(i):
        return (t_hit + 1 + i) % NT

    def out_tile(i, y, side=iter(())):
        t = tile_of(i)
        rs = pl.ds(pl.multiple_of(t * T, T), T)
        pn = jnp.concatenate([pn_v[g, rs, :] for g in range(NG)], axis=1)
        gate = gcol_v[rs, :]
        a = jnp.dot(pn, m_v[...].reshape(D, D), preferred_element_type=F32)
        for j in range(D // LANES):
            sl = slice(j * LANES, (j + 1) * LANES)
            xf = x_v[rs, sl].astype(F32)
            upd = xf * 0.0
            if y is not None:
                hit = lax.broadcasted_iota(jnp.int32, (T, LANES), 0) == idx - t * T
                upd = upd + jnp.where(hit, y[:, sl], 0.0)
            _advance(side, SO)
            ob_v[i % NB, :, sl] = (gate * a[:, sl] + (1.0 - gate) * (xf + upd)).astype(BF16)
        _advance(side, F)
        (o_copy if y is None else o_last)(i, t).start()

    def out_step(i):
        if isinstance(i, int):
            if i >= NB:
                o_copy(i - NB, tile_of(i - NB)).wait()
        else:
            @pl.when(i >= NB)
            def _():
                o_copy(i - NB, tile_of(i - NB)).wait()
        out_tile(i, None, ffn_down(i))

    def out_body(ii, carry):
        for u in range(UN):
            out_step(ii * UN + u)
        return carry

    for i in range(ND):
        d_copy(i).wait()
    n_loop = (NT - 1) // UN if UN < NT else 0
    if n_loop:
        lax.fori_loop(0, n_loop, out_body, 0)
    for i in range(n_loop * UN, NT - 1):
        out_step(i)
    o_copy(NT - 1 - NB, tile_of(NT - 1 - NB)).wait()
    out_tile(NT - 1, jnp.sum(y_v[...], axis=0, keepdims=True) * w_sel)
    for i in range(NT - NB, NT - 1):
        o_copy(i, tile_of(i)).wait()
    o_last(NT - 1, tile_of(NT - 1)).wait()


@jax.jit
def pallas_gated_mix__linear_attn_block__moe_arch_mod__prompt_kernel(
    A_x: jax.Array,
    A_wqkv: jax.Array,
    A_wo: jax.Array,
    B_x: jax.Array,
    B_w_r: jax.Array,
    B_w_gate: jax.Array,
    B_w_up: jax.Array,
    B_w_down: jax.Array,
    gate_w: jax.Array,
):
    del B_x
    hbm = pl.BlockSpec(memory_space=pl.ANY)
    vmem = pl.BlockSpec(memory_space=pltpu.VMEM)
    out = pl.pallas_call(
        _kernel,
        out_shape=jax.ShapeDtypeStruct((S, D), BF16),
        in_specs=[hbm, hbm, hbm, vmem, vmem, hbm, hbm, hbm],
        out_specs=hbm,
        scratch_shapes=[
            pltpu.VMEM((S, D), BF16),
            pltpu.VMEM((NG, D, G), BF16),
            pltpu.VMEM((NG, D, G), BF16),
            pltpu.VMEM((NG, D, G), BF16),
            pltpu.VMEM((NG, G, D), BF16),
            pltpu.VMEM((NF, D, FT * LANES), BF16),
            pltpu.VMEM((NF, D, FT * LANES), BF16),
            pltpu.VMEM((ND, FD, D), BF16),
            pltpu.VMEM((2 * G + XR, D), BF16),
            pltpu.VMEM((G, S), BF16),
            pltpu.VMEM((G, X0[-2]), F32),
            pltpu.VMEM((G, D), BF16),
            pltpu.VMEM((NG, S, G), BF16),
            pltpu.VMEM((NG, G, D), BF16),
            pltpu.VMEM((S, LANES), F32),
            pltpu.VMEM((D, LANES), F32),
            pltpu.VMEM((ND * FD // LANES, 16, LANES), F32),
            pltpu.VMEM((FD, LANES), F32),
            pltpu.VMEM((8, D), F32),
            pltpu.VMEM((8, S), F32),
            pltpu.VMEM((NB, T, D), BF16),
            pltpu.VMEM((8, LANES), jnp.int32),
            pltpu.SMEM((1,), jnp.int32),
            pltpu.SemaphoreType.DMA(((len(X0) - 1) * SX,)),
            pltpu.SemaphoreType.DMA((2 * SW,)),
            pltpu.SemaphoreType.DMA((4 * NG,)),
            pltpu.SemaphoreType.DMA((2 * NF + ND,)),
            pltpu.SemaphoreType.DMA((NB + SL,)),
        ],
        compiler_params=pltpu.CompilerParams(vmem_limit_bytes=110 * 1024 * 1024),
    )(A_x.reshape(S, D), A_wqkv, A_wo, B_w_r, gate_w,
      B_w_gate, B_w_up, B_w_down)
    return out.reshape(A_x.shape)
```

```python
import functools

import jax
import jax.numpy as jnp
from jax import lax
import jax.experimental.pallas as pl
import jax.experimental.pallas.tpu as pltpu

S, D, F = 2048, 1024, 3584
DH = 32
G = 256
NG = D // G
CS = 512
NC = S // CS
PN = 256
import os
RB = 128
NRB = S // RB
TB = int(os.environ.get('TB', 3))
NT = (NRB - 1) // TB
XR = 16
LANES = 128
FT, FS = 10, 9
NF = NG - 1
ND = NT
FD = -(-F // (ND * LANES)) * LANES
import os
X0 = tuple(int(v) for v in os.environ.get('X0', '0,256,512,1024,2048').split(','))

import os
PU = int(os.environ.get('PU', 2)); PK = int(os.environ.get('PK', 1)); PJ = int(os.environ.get('PJ', 4))
SK = int(os.environ.get('SK', 10)); SP = int(os.environ.get('SP', 20)); SO = int(os.environ.get('SO', 8)); ACT = int(os.environ.get('ACT', 3))
SU = int(os.environ.get('SU', 2)); SD = int(os.environ.get('SD', 4))
UN = int(os.environ.get('UN', 1)); NB = int(os.environ.get('NB', 2))
SX = int(os.environ.get('SX', 1)); SW = int(os.environ.get('SW', 1)); SL = int(os.environ.get('SL', 1))
DA = int(os.environ.get('DA', 20)); GT = int(os.environ.get('GT', 1)); MR = int(os.environ.get('MR', 0)); MC = int(os.environ.get('MC', 384))
TK = int(os.environ.get('TK', 1))
_NT = (((1,), (1,)), ((), ()))
F32, BF16 = jnp.float32, jnp.bfloat16


def _phi(t):
    return jnp.where(t > 0, t + 1.0, jnp.exp(t)) + 1e-6


def _sigmoid(t):
    return 1.0 / (1.0 + jnp.exp(-t))


def _lane_tile_sum(v):
    acc = v[:, 0:LANES]
    for j in range(1, v.shape[1] // LANES):
        acc = acc + v[:, j * LANES:(j + 1) * LANES]
    return acc


def _to_cols(row):
    return jnp.broadcast_to(row, (LANES, row.shape[1])).T


def _advance(steps, n):
    for _ in range(n):
        next(steps, None)


class _Split:
    def __init__(self, src, dst, sems, base, parts):
        n = src.shape[0] // parts
        self.copies = [pltpu.make_async_copy(src.at[pl.ds(i * n, n)], dst.at[pl.ds(i * n, n)],
                                             sems.at[base + i]) for i in range(parts)]

    def start(self):
        for cp in self.copies:
            cp.start()

    def wait(self):
        for cp in self.copies:
            cp.wait()


def _bits(v):
    return pltpu.bitcast(v, jnp.int32)


def _fold(v, delay=0):
    v = _bits(v)
    v = functools.reduce(jnp.bitwise_or, [v[:, j:j + LANES] for j in range(0, v.shape[1], LANES)])
    v = functools.reduce(jnp.bitwise_or, [v[i:i + 8] for i in range(0, v.shape[0], 8)])
    v = pltpu.bitcast(v, F32)
    for _ in range(delay):
        v = pl.reciprocal(v, approx=True)
    return _bits(v)


def _kernel(x_hbm, wqkv_hbm, wo_hbm, wr_ref, gw_ref, wg_hbm, wu_hbm, wd_hbm, out_hbm,
            x_v, wq_v, wk_v, wv_v, wo_v, wg_v, wu_v, wd_v,
            wt_v, pk_v, pq_v, p_v, pn_v, m_v, gcol_v, xcol_v, h_v, hcol_v, y_v, rg_v, ob_v, zero_v,
            idx_s, sem_x, sem_0, sem_w, sem_f, sem_o):

    def x_copy(c):
        rs = pl.ds(X0[c], X0[c + 1] - X0[c])
        return _Split(x_hbm.at[rs], x_v.at[rs], sem_x, c * SX, SX)

    def w0_copy(kind):
        return _Split(wqkv_hbm.at[:, pl.ds(kind * D, G)], (wq_v, wk_v)[kind].at[0], sem_0, kind * SW, SW)

    def w_copy(kind, g):
        off = g * G if isinstance(g, int) else pl.multiple_of(g * G, G)
        if kind == 3:
            return pltpu.make_async_copy(wo_hbm.at[pl.ds(off, G)], wo_v.at[g], sem_w.at[3 * NG + g])
        return pltpu.make_async_copy(wqkv_hbm.at[:, pl.ds(kind * D + off, G)],
                                     (wq_v, wk_v, wv_v)[kind].at[g], sem_w.at[kind * NG + g])

    def f_copy(kind, c):
        off = c * FS * LANES
        sl = pl.ds(off if isinstance(c, int) else pl.multiple_of(off, LANES), FT * LANES)
        return pltpu.make_async_copy((wg_hbm, wu_hbm)[kind].at[:, sl], (wg_v, wu_v)[kind].at[c],
                                     sem_f.at[kind * NF + c])

    def d_copy(i):
        n = min(FD, F - i * FD)
        return pltpu.make_async_copy(wd_hbm.at[pl.ds(i * FD, n)], wd_v.at[i, pl.ds(0, n)],
                                     sem_f.at[2 * NF + i])

    def after(lhs, token):
        if token is None:
            return lhs
        t = token & zero_v[...]
        top = _bits(lhs[0:16]) | jnp.concatenate([t] * (lhs.shape[1] // LANES), axis=1)
        return jnp.concatenate([pltpu.bitcast(top, BF16), lhs[16:]], axis=0)

    def project(lhs, rs):
        return lax.dot_general(lhs, x_v[rs, :], _NT, preferred_element_type=F32)

    def p_part(n, token, side=iter(())):
        p = jnp.dot(after(pk_v[...], token), x_v[:, n * PN:(n + 1) * PN], preferred_element_type=F32)
        for j in range(0, PN, LANES):
            _advance(side, SP)
            p_v[:, n * PN + j:n * PN + j + LANES] = p[:, j:j + LANES].astype(BF16)

    def normalize(g, rs, pq, z):
        n = pq.shape[1]
        pq = pq.reshape(G // DH, DH, n)
        den = jnp.sum(pq * z, axis=1, keepdims=True) + 1e-6
        pn = (pq * (1.0 / den)).reshape(G, n).astype(BF16).T
        pn_v[g, rs, :] = pn
        return pn

    def kv_part(g):
        ri = lax.broadcasted_iota(jnp.int32, (LANES, LANES), 0) // DH
        ci = lax.broadcasted_iota(jnp.int32, (LANES, LANES), 1) // DH
        out = []
        for j in range(G // LANES):
            sl = slice(j * LANES, (j + 1) * LANES)
            kv = jnp.dot(p_v[sl, :], wv_v[g, :, sl], preferred_element_type=F32)
            out.append(jnp.where(ri == ci, kv, 0.0).astype(BF16))
        return out

    def m_part(g, kvs, token=None):
        for j, kv in enumerate(kvs):
            sl = slice(j * LANES, (j + 1) * LANES)
            m_v[g, sl, :] = jnp.dot(after(kv, token), wo_v[g, sl, :], preferred_element_type=F32).astype(BF16)

    def route():
        r = rg_v[0:1, :].astype(BF16).astype(F32)
        pos = lax.broadcasted_iota(jnp.int32, (1, S), 1)
        valid = r == r
        rmax = jnp.max(jnp.where(valid, r, -jnp.inf), axis=1, keepdims=True)
        cand = jnp.logical_and(valid, r == rmax)
        idxv = jnp.min(jnp.where(cand, pos, S).astype(F32), axis=1, keepdims=True).astype(jnp.int32)
        idxv = jnp.where(idxv >= S, 0, idxv)
        r_sel = jnp.sum(jnp.where(pos == idxv, r, 0.0), axis=1, keepdims=True)
        idx = idxv[0, 0]
        idx_s[0] = idx
        base = pl.multiple_of(jnp.clip((idx // 16) * 16, 0, S - 16), 16)
        rows = x_v[pl.ds(base, 16), :].astype(F32)
        rid = lax.broadcasted_iota(jnp.int32, (16, D), 0)
        x_sel = jnp.sum(jnp.where(rid == idx - base, rows, 0.0), axis=0, keepdims=True)
        xcol_v[...] = _to_cols(x_sel)
        return _sigmoid(r_sel)

    def matvec(col_ref, nk, tiles, accs, slow):
        keep = zero_v[...] == 0
        for k in range(0, nk, 16):
            lo, hi = col_ref[k:k + 8, :], col_ref[k + 8:k + 16, :]
            if k % (16 * PK) == 0 and accs[-1] is not None:
                t = accs[-1]
                for _ in range(slow):
                    t = pl.reciprocal(t, approx=True)
                lo, hi = jnp.where(keep, lo, t), jnp.where(keep, hi, t)
            for j, (w_ref, r0, c0) in enumerate(tiles):
                w = w_ref[r0 + k:r0 + k + 16, c0:c0 + LANES].astype(F32)
                p = w[0:8] * lo + w[8:16] * hi
                accs[j] = p if accs[j] is None else accs[j] + p
            yield

    def ffn_up(c):
        for i in range(0, FT, PU):
            accs = [None] * (2 * PU)
            yield from matvec(xcol_v, D, [(w.at[c], 0, (i + u) * LANES)
                                          for u in range(PU) for w in (wg_v, wu_v)], accs, SU)
            for u in range(PU):
                h_v[c * FS + i + u, 0:8, :] = accs[2 * u]
                h_v[c * FS + i + u, 8:16, :] = accs[2 * u + 1]

    def ffn_down(i):
        for u in range(FD // LANES):
            hg = jnp.sum(h_v[i * (FD // LANES) + u, 0:8, :], axis=0, keepdims=True)
            hu = jnp.sum(h_v[i * (FD // LANES) + u, 8:16, :], axis=0, keepdims=True)
            hcol_v[u * LANES:(u + 1) * LANES, :] = _to_cols(hg * _sigmoid(hg) * hu)
        for j0 in range(0, D, LANES * PJ):
            cols = range(j0, j0 + LANES * PJ, LANES)
            accs = [y_v[:, j:j + LANES] for j in cols]
            yield from matvec(hcol_v, FD, [(wd_v.at[i], 0, j) for j in cols], accs, SD)
            for j, acc in zip(cols, accs):
                y_v[:, j:j + LANES] = acc

    nx = len(X0) - 1
    w0_copy(1).start()
    x_copy(0).start()
    w0_copy(0).start()
    x_copy(1).start()
    wt_v[2 * G:2 * G + XR, :] = jnp.concatenate(
        [wr_ref[...].astype(F32).reshape(1, D), gw_ref[...].astype(F32).reshape(1, D),
         jnp.zeros((XR - 2, D), F32)], axis=0).astype(BF16)
    y_v[...] = jnp.zeros(y_v.shape, F32)
    if ND * FD > F:
        wd_v[ND - 1, F - (ND - 1) * FD:, :] = jnp.zeros((ND * FD - F, D), BF16)
        h_v[F // LANES:] = jnp.zeros(((ND * FD - F) // LANES, 16, LANES), F32)
    zero_v[...] = jnp.zeros(zero_v.shape, jnp.int32)
    w0_copy(1).wait()
    wt_v[G:2 * G, :] = wk_v[0].T
    first = [w_copy(2, 0), w_copy(3, 0), w_copy(1, 1)]
    zacc = None
    for c in range(nx):
        rs = slice(X0[c], X0[c + 1])
        x_copy(c).wait()
        if c == 0:
            for cc in range(2, nx):
                x_copy(cc).start()
        if c == nx - 1:
            for cp in (first + [w_copy(k, 1) for k in (0, 2, 3)] + [w_copy(1, 2)]
                       + [f_copy(k, 0) for k in range(2)]):
                cp.start()
        if c == 0:
            k = project(wt_v[G:2 * G + XR, :], rs)
            w0_copy(0).wait()
            wt_v[0:G, :] = wq_v[0].T
            q = project(wt_v[0:G, :], rs)
        elif c < nx - 1:
            qk = project(wt_v[...], rs)
            q, k = qk[0:G], qk[G:]
        else:
            q, k = None, project(wt_v[G:2 * G + XR, :], rs)
        pk = _phi(k[0:G])
        pk_v[:, rs] = pk.astype(BF16)
        if q is not None:
            pq_v[:, rs] = _phi(q)
        rg_v[:, rs] = k[G:G + 8]
        zc = _lane_tile_sum(pk)
        zacc = zc if zacc is None else zacc + zc
    for cp in first:
        cp.wait()
    z = jnp.sum(zacc, axis=1, keepdims=True).reshape(G // DH, DH, 1)
    token = None
    for n in range(D // PN):
        p_part(n, token)
        rs = slice(n * CS, (n + 1) * CS)
        if n == 0:
            w_sel = route()
        gcol_v[rs, :] = _to_cols(_sigmoid(rg_v[1:2, rs]))
        token = None
        if (n + 1) * CS <= X0[nx - 1]:
            pn = normalize(0, rs, pq_v[:, rs], z)
            if TK:
                token = _bits(pn[CS - 16:, G - LANES:])
    wt_v[G:2 * G, :] = wk_v[1].T
    kvs = kv_part(0)
    for r0 in range(X0[nx - 1], S, CS):
        rs = slice(r0, r0 + CS)
        q = project(wt_v[0:G, :], rs)
        normalize(0, rs, _phi(q), z)
    m_part(0, kvs, _bits(q[MR:MR + 8, MC:MC + LANES]))

    def group_body(g, carry):
        nxt = jnp.minimum(g + 1, NG - 1)

        @pl.when(g + 1 < NG)
        def _():
            for kind in (0, 2, 3):
                w_copy(kind, g + 1).start()
            for kind in range(2):
                f_copy(kind, g).start()

        @pl.when(g + 2 < NG)
        def _():
            w_copy(1, g + 2).start()

        @pl.when(g == NG - 1)
        def _():
            for i in range(ND):
                d_copy(i).start()
        for kind in (0, 2, 3):
            w_copy(kind, g).wait()
        for kind in range(2):
            f_copy(kind, g - 1).wait()

        @pl.when(g + 1 < NG)
        def _():
            w_copy(1, g + 1).wait()

        side = ffn_up(g - 1)
        zacc = None
        for c in range(NC):
            k = project(wt_v[G:2 * G, :], slice(c * CS, (c + 1) * CS))
            for j in range(0, CS, LANES):
                pk = _phi(k[:, j:j + LANES])
                _advance(side, SK)
                pk_v[:, c * CS + j:c * CS + j + LANES] = pk.astype(BF16)
                zacc = pk if zacc is None else zacc + pk
        z = jnp.sum(zacc, axis=1, keepdims=True).reshape(G // DH, DH, 1)
        wt_v[0:G, :] = wq_v[g].T
        for n in range(D // PN):
            p_part(n, None, side)
        _advance(side, FT * D)
        wt_v[G:2 * G, :] = wk_v[nxt].T
        for c in range(NC):
            rs = slice(c * CS, (c + 1) * CS)
            q = project(wt_v[0:G, :], rs)
            normalize(g, rs, _phi(q), z)
            if c == 1:
                kvs = kv_part(g)
            if c == NC - 1:
                m_part(g, kvs, _bits(q[MR:MR + 8, MC:MC + LANES]) if MC >= 0 else None)
        return carry

    lax.fori_loop(1, NG, group_body, 0)

    idx = idx_s[0]
    b_hit = jnp.clip(idx // RB, 0, NRB - 1)

    def rows_of(n):
        return pl.ds(pl.multiple_of((b_hit + 1 + n) % NRB * RB, RB), RB)

    def o_copy(n, slot):
        return pltpu.make_async_copy(ob_v.at[slot], out_hbm.at[rows_of(n)], sem_o.at[slot])

    def out_blocks(n0, count, slot0, upd):
        pn = jnp.concatenate(
            [jnp.concatenate([pn_v[g, rows_of(n0 + j), :] for g in range(NG)], axis=1)
             for j in range(count)], axis=0)
        a = jnp.dot(pn, m_v[...].reshape(D, D), preferred_element_type=F32)
        for j in range(count):
            rs = rows_of(n0 + j)
            gate = gcol_v[rs, :]
            for c0 in range(0, D, LANES):
                sl = slice(c0, c0 + LANES)
                xf = x_v[rs, sl].astype(F32)
                b = xf + (xf * 0.0 if upd is None else xf * 0.0 + upd(sl))
                ob_v[slot0 + j, :, sl] = (gate * a[j * RB:(j + 1) * RB, sl]
                                          + (1.0 - gate) * b).astype(BF16)
        for j in range(count):
            o_copy(n0 + j, slot0 + j).start()

    def out_wait(i):
        for j in range(TB):
            o_copy(i * TB + j, i % 2 * TB + j).wait()

    def out_body(i, carry):
        pl.when(i >= 2)(lambda: out_wait(i - 2))
        for _ in ffn_down(i):
            pass
        out_blocks(i * TB, TB, i % 2 * TB, None)
        return carry

    for i in range(ND):
        d_copy(i).wait()
    lax.fori_loop(0, NT, out_body, 0)
    y = jnp.sum(y_v[...], axis=0, keepdims=True) * w_sel
    hit = lax.broadcasted_iota(jnp.int32, (RB, LANES), 0) == idx - b_hit * RB
    out_blocks(NRB - 1, 1, 2 * TB, lambda sl: jnp.where(hit, y[:, sl], 0.0))
    out_wait(NT - 2)
    out_wait(NT - 1)
    o_copy(NRB - 1, 2 * TB).wait()


@jax.jit
def pallas_gated_mix__linear_attn_block__moe_arch_mod__prompt_kernel(
    A_x: jax.Array,
    A_wqkv: jax.Array,
    A_wo: jax.Array,
    B_x: jax.Array,
    B_w_r: jax.Array,
    B_w_gate: jax.Array,
    B_w_up: jax.Array,
    B_w_down: jax.Array,
    gate_w: jax.Array,
):
    del B_x
    hbm = pl.BlockSpec(memory_space=pl.ANY)
    vmem = pl.BlockSpec(memory_space=pltpu.VMEM)
    out = pl.pallas_call(
        _kernel,
        out_shape=jax.ShapeDtypeStruct((S, D), BF16),
        in_specs=[hbm, hbm, hbm, vmem, vmem, hbm, hbm, hbm],
        out_specs=hbm,
        scratch_shapes=[
            pltpu.VMEM((S, D), BF16),
            pltpu.VMEM((NG, D, G), BF16),
            pltpu.VMEM((NG, D, G), BF16),
            pltpu.VMEM((NG, D, G), BF16),
            pltpu.VMEM((NG, G, D), BF16),
            pltpu.VMEM((NF, D, FT * LANES), BF16),
            pltpu.VMEM((NF, D, FT * LANES), BF16),
            pltpu.VMEM((ND, FD, D), BF16),
            pltpu.VMEM((2 * G + XR, D), BF16),
            pltpu.VMEM((G, S), BF16),
            pltpu.VMEM((G, X0[-2]), F32),
            pltpu.VMEM((G, D), BF16),
            pltpu.VMEM((NG, S, G), BF16),
            pltpu.VMEM((NG, G, D), BF16),
            pltpu.VMEM((S, LANES), F32),
            pltpu.VMEM((D, LANES), F32),
            pltpu.VMEM((ND * FD // LANES, 16, LANES), F32),
            pltpu.VMEM((FD, LANES), F32),
            pltpu.VMEM((8, D), F32),
            pltpu.VMEM((8, S), F32),
            pltpu.VMEM((2 * TB + 1, RB, D), BF16),
            pltpu.VMEM((8, LANES), jnp.int32),
            pltpu.SMEM((1,), jnp.int32),
            pltpu.SemaphoreType.DMA(((len(X0) - 1) * SX,)),
            pltpu.SemaphoreType.DMA((2 * SW,)),
            pltpu.SemaphoreType.DMA((4 * NG,)),
            pltpu.SemaphoreType.DMA((2 * NF + ND,)),
            pltpu.SemaphoreType.DMA((2 * TB + 1,)),
        ],
        compiler_params=pltpu.CompilerParams(vmem_limit_bytes=110 * 1024 * 1024),
    )(A_x.reshape(S, D), A_wqkv, A_wo, B_w_r, gate_w,
      B_w_gate, B_w_up, B_w_down)
    return out.reshape(A_x.shape)
```

```python
import jax
import jax.numpy as jnp
from jax import lax
import jax.experimental.pallas as pl
import jax.experimental.pallas.tpu as pltpu

S, D, F = 2048, 1024, 3584
DH = 32
LANES = 128
G = 256
NG = D // G
CS = 512
PN = 256
XR = 16
X0 = (0, 256, 512, 1024, 2048)
NX = len(X0) - 1
FT, FS = 10, 9
NF = NG - 1
RB = 128
NRB = S // RB
TB = 3
NT = (NRB - 1) // TB
FD = -(-F // (NT * LANES)) * LANES

_NT = (((1,), (1,)), ((), ()))
F32, BF16 = jnp.float32, jnp.bfloat16
Q, K, V, O = range(4)
GATE, UP = range(2)


def _phi(t):
    return jnp.where(t > 0, t + 1.0, jnp.exp(t)) + 1e-6


def _sigmoid(t):
    return 1.0 / (1.0 + jnp.exp(-t))


def _lane_tile_sum(v):
    acc = v[:, 0:LANES]
    for j in range(LANES, v.shape[1], LANES):
        acc = acc + v[:, j:j + LANES]
    return acc


def _to_cols(row):
    return jnp.broadcast_to(row, (LANES, row.shape[1])).T


def _bits(v):
    return pltpu.bitcast(v, jnp.int32)


def _aligned(i, n):
    return i if isinstance(i, int) else pl.multiple_of(i, n)


def _kernel(x_hbm, wqkv_hbm, wo_hbm, wr_ref, gw_ref, wg_hbm, wu_hbm, wd_hbm, out_hbm,
            x_v, wq_v, wk_v, wv_v, wo_v, wg_v, wu_v, wd_v,
            wt_v, pk_v, pq_v, p_v, pn_v, m_v, gcol_v, xcol_v, h_v, hcol_v, y_v, rg_v, ob_v, zero_v,
            idx_s, sem_x, sem_w, sem_f, sem_d, sem_o):

    def x_copy(c):
        rs = pl.ds(X0[c], X0[c + 1] - X0[c])
        return pltpu.make_async_copy(x_hbm.at[rs], x_v.at[rs], sem_x.at[c])

    def w_copy(kind, g):
        sem = sem_w.at[kind * NG + g]
        if kind == O:
            return pltpu.make_async_copy(wo_hbm.at[pl.ds(_aligned(g * G, G), G)], wo_v.at[g], sem)
        cols = pl.ds(_aligned(kind * D + g * G, G), G)
        return pltpu.make_async_copy(wqkv_hbm.at[:, cols], (wq_v, wk_v, wv_v)[kind].at[g], sem)

    def f_copy(kind, c):
        cols = pl.ds(_aligned(c * FS * LANES, LANES), FT * LANES)
        return pltpu.make_async_copy((wg_hbm, wu_hbm)[kind].at[:, cols], (wg_v, wu_v)[kind].at[c],
                                     sem_f.at[kind * NF + c])

    def d_copy(i):
        n = min(FD, F - i * FD)
        return pltpu.make_async_copy(wd_hbm.at[pl.ds(i * FD, n)], wd_v.at[i, pl.ds(0, n)],
                                     sem_d.at[i])

    def after(lhs, token):
        if token is None:
            return lhs
        t = token & zero_v[...]
        top = _bits(lhs[0:16]) | jnp.concatenate([t] * (lhs.shape[1] // LANES), axis=1)
        return jnp.concatenate([pltpu.bitcast(top, BF16), lhs[16:]], axis=0)

    def matvec(col_ref, nk, tiles, accs, delay):
        keep = zero_v[...] == 0
        for k in range(0, nk, 16):
            lo, hi = col_ref[k:k + 8, :], col_ref[k + 8:k + 16, :]
            if accs[-1] is not None:
                t = accs[-1]
                for _ in range(delay):
                    t = pl.reciprocal(t, approx=True)
                lo, hi = jnp.where(keep, lo, t), jnp.where(keep, hi, t)
            for j, (w_ref, c0) in enumerate(tiles):
                w = w_ref[k:k + 16, c0:c0 + LANES].astype(F32)
                p = w[0:8] * lo + w[8:16] * hi
                accs[j] = p if accs[j] is None else accs[j] + p
        return accs

    def project(lhs, rs):
        return lax.dot_general(lhs, x_v[rs, :], _NT, preferred_element_type=F32)

    def p_part(n, token=None):
        ns = slice(n * PN, (n + 1) * PN)
        p_v[:, ns] = jnp.dot(after(pk_v[...], token), x_v[:, ns],
                             preferred_element_type=F32).astype(BF16)

    def normalize(g, rs, pq, z):
        n = pq.shape[1]
        pq = pq.reshape(G // DH, DH, n)
        den = jnp.sum(pq * z, axis=1, keepdims=True) + 1e-6
        pn = (pq * (1.0 / den)).reshape(G, n).astype(BF16).T
        pn_v[g, rs, :] = pn
        return pn

    def kv_part(g):
        ri = lax.broadcasted_iota(jnp.int32, (LANES, LANES), 0) // DH
        ci = lax.broadcasted_iota(jnp.int32, (LANES, LANES), 1) // DH
        kvs = []
        for j in range(0, G, LANES):
            kv = jnp.dot(p_v[j:j + LANES, :], wv_v[g, :, j:j + LANES], preferred_element_type=F32)
            kvs.append(jnp.where(ri == ci, kv, 0.0).astype(BF16))
        return kvs

    def m_part(g, kvs, last_q):
        token = _bits(last_q[0:8, CS - LANES:])
        for j, kv in zip(range(0, G, LANES), kvs):
            m_v[g, j:j + LANES, :] = jnp.dot(after(kv, token), wo_v[g, j:j + LANES, :],
                                             preferred_element_type=F32).astype(BF16)

    def route():
        r = rg_v[0:1, :].astype(BF16).astype(F32)
        pos = lax.broadcasted_iota(jnp.int32, (1, S), 1)
        valid = r == r
        rmax = jnp.max(jnp.where(valid, r, -jnp.inf), axis=1, keepdims=True)
        cand = jnp.logical_and(valid, r == rmax)
        idxv = jnp.min(jnp.where(cand, pos, S).astype(F32), axis=1, keepdims=True).astype(jnp.int32)
        idxv = jnp.where(idxv >= S, 0, idxv)
        r_sel = jnp.sum(jnp.where(pos == idxv, r, 0.0), axis=1, keepdims=True)
        idx = idxv[0, 0]
        idx_s[0] = idx
        base = pl.multiple_of(jnp.clip((idx // 16) * 16, 0, S - 16), 16)
        rows = x_v[pl.ds(base, 16), :].astype(F32)
        rid = lax.broadcasted_iota(jnp.int32, (16, D), 0)
        x_sel = jnp.sum(jnp.where(rid == idx - base, rows, 0.0), axis=0, keepdims=True)
        xcol_v[...] = _to_cols(x_sel)
        return _sigmoid(r_sel)

    def ffn_up(c):
        for i in range(0, FT, 2):
            tiles = [(w.at[c], (i + u) * LANES) for u in range(2) for w in (wg_v, wu_v)]
            accs = matvec(xcol_v, D, tiles, [None] * 4, 2)
            for u in range(2):
                h_v[c * FS + i + u, 0:8, :] = accs[2 * u]
                h_v[c * FS + i + u, 8:16, :] = accs[2 * u + 1]

    def ffn_down(i):
        for u in range(FD // LANES):
            hg = jnp.sum(h_v[i * (FD // LANES) + u, 0:8, :], axis=0, keepdims=True)
            hu = jnp.sum(h_v[i * (FD // LANES) + u, 8:16, :], axis=0, keepdims=True)
            hcol_v[u * LANES:(u + 1) * LANES, :] = _to_cols(hg * _sigmoid(hg) * hu)
        for j0 in range(0, D, 4 * LANES):
            cols = range(j0, j0 + 4 * LANES, LANES)
            accs = matvec(hcol_v, FD, [(wd_v.at[i], j) for j in cols],
                          [y_v[:, j:j + LANES] for j in cols], 4)
            for j, acc in zip(cols, accs):
                y_v[:, j:j + LANES] = acc

    for cp in (w_copy(K, 0), x_copy(0), w_copy(Q, 0), x_copy(1)):
        cp.start()
    wt_v[2 * G:2 * G + XR, :] = jnp.concatenate(
        [wr_ref[...].astype(F32).reshape(1, D), gw_ref[...].astype(F32).reshape(1, D),
         jnp.zeros((XR - 2, D), F32)], axis=0).astype(BF16)
    y_v[...] = jnp.zeros(y_v.shape, F32)
    zero_v[...] = jnp.zeros(zero_v.shape, jnp.int32)
    wd_v[NT - 1, F - (NT - 1) * FD:, :] = jnp.zeros((NT * FD - F, D), BF16)
    h_v[F // LANES:] = jnp.zeros(((NT * FD - F) // LANES, 16, LANES), F32)
    w_copy(K, 0).wait()
    wt_v[G:2 * G, :] = wk_v[0].T

    first = [w_copy(V, 0), w_copy(O, 0), w_copy(K, 1)]
    zacc = None
    for c in range(NX):
        rs = slice(X0[c], X0[c + 1])
        x_copy(c).wait()
        if c == 0:
            for cc in range(2, NX):
                x_copy(cc).start()
        if c == NX - 1:
            for cp in first + [w_copy(Q, 1), w_copy(V, 1), w_copy(O, 1), w_copy(K, 2),
                               f_copy(GATE, 0), f_copy(UP, 0)]:
                cp.start()
        if c == 0:
            k = project(wt_v[G:, :], rs)
            w_copy(Q, 0).wait()
            wt_v[0:G, :] = wq_v[0].T
            q = project(wt_v[0:G, :], rs)
        elif c < NX - 1:
            qk = project(wt_v[...], rs)
            q, k = qk[0:G], qk[G:]
        else:
            q, k = None, project(wt_v[G:, :], rs)
        pk = _phi(k[0:G])
        pk_v[:, rs] = pk.astype(BF16)
        if q is not None:
            pq_v[:, rs] = _phi(q)
        rg_v[:, rs] = k[G:G + 8]
        zc = _lane_tile_sum(pk)
        zacc = zc if zacc is None else zacc + zc
    for cp in first:
        cp.wait()
    z = jnp.sum(zacc, axis=1, keepdims=True).reshape(G // DH, DH, 1)
    token = None
    for n in range(D // PN):
        p_part(n, token)
        rs = slice(n * CS, (n + 1) * CS)
        if n == 0:
            w_sel = route()
        gcol_v[rs, :] = _to_cols(_sigmoid(rg_v[1:2, rs]))
        token = None
        if (n + 1) * CS <= X0[NX - 1]:
            token = _bits(normalize(0, rs, pq_v[:, rs], z)[CS - 16:, G - LANES:])
    wt_v[G:2 * G, :] = wk_v[1].T
    kvs = kv_part(0)
    for r0 in range(X0[NX - 1], S, CS):
        rs = slice(r0, r0 + CS)
        q = project(wt_v[0:G, :], rs)
        normalize(0, rs, _phi(q), z)
    m_part(0, kvs, q)

    def group_body(g, carry):
        @pl.when(g + 1 < NG)
        def _():
            for kind in (Q, V, O):
                w_copy(kind, g + 1).start()
            for kind in (GATE, UP):
                f_copy(kind, g).start()

        @pl.when(g + 2 < NG)
        def _():
            w_copy(K, g + 2).start()

        @pl.when(g == NG - 1)
        def _():
            for i in range(NT):
                d_copy(i).start()

        for kind in (Q, V, O):
            w_copy(kind, g).wait()
        for kind in (GATE, UP):
            f_copy(kind, g - 1).wait()

        @pl.when(g + 1 < NG)
        def _():
            w_copy(K, g + 1).wait()

        ffn_up(g - 1)
        zacc = None
        for r0 in range(0, S, CS):
            k = project(wt_v[G:2 * G, :], slice(r0, r0 + CS))
            for j in range(0, CS, LANES):
                pk = _phi(k[:, j:j + LANES])
                pk_v[:, r0 + j:r0 + j + LANES] = pk.astype(BF16)
                zacc = pk if zacc is None else zacc + pk
        z = jnp.sum(zacc, axis=1, keepdims=True).reshape(G // DH, DH, 1)
        wt_v[0:G, :] = wq_v[g].T
        for n in range(D // PN):
            p_part(n)
        wt_v[G:2 * G, :] = wk_v[jnp.minimum(g + 1, NG - 1)].T
        kvs = kv_part(g)
        for r0 in range(0, S, CS):
            rs = slice(r0, r0 + CS)
            q = project(wt_v[0:G, :], rs)
            normalize(g, rs, _phi(q), z)
        m_part(g, kvs, q)
        return carry

    lax.fori_loop(1, NG, group_body, 0)

    idx = idx_s[0]
    b_hit = jnp.clip(idx // RB, 0, NRB - 1)

    def rows_of(n):
        return pl.ds(pl.multiple_of((b_hit + 1 + n) % NRB * RB, RB), RB)

    def o_copy(n, slot):
        return pltpu.make_async_copy(ob_v.at[slot], out_hbm.at[rows_of(n)], sem_o.at[slot])

    def out_blocks(n0, count, slot0, update):
        pn = jnp.concatenate(
            [jnp.concatenate([pn_v[g, rows_of(n0 + j), :] for g in range(NG)], axis=1)
             for j in range(count)], axis=0)
        a = jnp.dot(pn, m_v[...].reshape(D, D), preferred_element_type=F32)
        for j in range(count):
            rs = rows_of(n0 + j)
            gate = gcol_v[rs, :]
            for c0 in range(0, D, LANES):
                sl = slice(c0, c0 + LANES)
                xf = x_v[rs, sl].astype(F32)
                b = xf + (xf * 0.0 if update is None else xf * 0.0 + update(sl))
                ob_v[slot0 + j, :, sl] = (gate * a[j * RB:(j + 1) * RB, sl]
                                          + (1.0 - gate) * b).astype(BF16)
        for j in range(count):
            o_copy(n0 + j, slot0 + j).start()

    def out_wait(i):
        for j in range(TB):
            o_copy(i * TB + j, i % 2 * TB + j).wait()

    def out_body(i, carry):
        @pl.when(i >= 2)
        def _():
            out_wait(i - 2)

        ffn_down(i)
        out_blocks(i * TB, TB, i % 2 * TB, None)
        return carry

    for i in range(NT):
        d_copy(i).wait()
    lax.fori_loop(0, NT, out_body, 0)
    y = jnp.sum(y_v[...], axis=0, keepdims=True) * w_sel
    hit = lax.broadcasted_iota(jnp.int32, (RB, LANES), 0) == idx - b_hit * RB
    out_blocks(NRB - 1, 1, 2 * TB, lambda sl: jnp.where(hit, y[:, sl], 0.0))
    out_wait(NT - 2)
    out_wait(NT - 1)
    o_copy(NRB - 1, 2 * TB).wait()


@jax.jit
def pallas_gated_mix__linear_attn_block__moe_arch_mod__prompt_kernel(
    A_x: jax.Array,
    A_wqkv: jax.Array,
    A_wo: jax.Array,
    B_x: jax.Array,
    B_w_r: jax.Array,
    B_w_gate: jax.Array,
    B_w_up: jax.Array,
    B_w_down: jax.Array,
    gate_w: jax.Array,
):
    del B_x
    hbm = pl.BlockSpec(memory_space=pl.ANY)
    vmem = pl.BlockSpec(memory_space=pltpu.VMEM)
    out = pl.pallas_call(
        _kernel,
        out_shape=jax.ShapeDtypeStruct((S, D), BF16),
        in_specs=[hbm, hbm, hbm, vmem, vmem, hbm, hbm, hbm],
        out_specs=hbm,
        scratch_shapes=[
            pltpu.VMEM((S, D), BF16),
            pltpu.VMEM((NG, D, G), BF16),
            pltpu.VMEM((NG, D, G), BF16),
            pltpu.VMEM((NG, D, G), BF16),
            pltpu.VMEM((NG, G, D), BF16),
            pltpu.VMEM((NF, D, FT * LANES), BF16),
            pltpu.VMEM((NF, D, FT * LANES), BF16),
            pltpu.VMEM((NT, FD, D), BF16),
            pltpu.VMEM((2 * G + XR, D), BF16),
            pltpu.VMEM((G, S), BF16),
            pltpu.VMEM((G, X0[NX - 1]), F32),
            pltpu.VMEM((G, D), BF16),
            pltpu.VMEM((NG, S, G), BF16),
            pltpu.VMEM((NG, G, D), BF16),
            pltpu.VMEM((S, LANES), F32),
            pltpu.VMEM((D, LANES), F32),
            pltpu.VMEM((NT * FD // LANES, 16, LANES), F32),
            pltpu.VMEM((FD, LANES), F32),
            pltpu.VMEM((8, D), F32),
            pltpu.VMEM((8, S), F32),
            pltpu.VMEM((2 * TB + 1, RB, D), BF16),
            pltpu.VMEM((8, LANES), jnp.int32),
            pltpu.SMEM((1,), jnp.int32),
            pltpu.SemaphoreType.DMA((NX,)),
            pltpu.SemaphoreType.DMA((4 * NG,)),
            pltpu.SemaphoreType.DMA((2 * NF,)),
            pltpu.SemaphoreType.DMA((NT,)),
            pltpu.SemaphoreType.DMA((2 * TB + 1,)),
        ],
        compiler_params=pltpu.CompilerParams(vmem_limit_bytes=110 * 1024 * 1024),
    )(A_x.reshape(S, D), A_wqkv, A_wo, B_w_r, gate_w, B_w_gate, B_w_up, B_w_down)
    return out.reshape(A_x.shape)
```
